```python
import jax
import jax.numpy as jnp

def _softmax(x, axis=-1):
    return jax.nn.softmax(x, axis=axis)

def _gelu(x):
    return jax.nn.gelu(x, approximate=True)

def _silu(x):
    return jax.nn.silu(x)

def _sigmoid(x):
    return jax.nn.sigmoid(x)

def _layernorm(x, axis=-1, eps=1e-05):
    m = jnp.mean(x, axis=axis, keepdims=True)
    v = jnp.var(x, axis=axis, keepdims=True)
    return (x - m) / jnp.sqrt(v + eps)

def _scatter_add(tgt, idx, src, axis=0):
    return tgt.at[idx].add(src)

def _segment_sum(src, seg, n):
    return jax.ops.segment_sum(src, seg, n)

class _Rng:

    def __init__(self, key):
        self._k = key

    def _next(self):
        self._k, sub = jax.random.split(self._k)
        return sub

    def normal(self, shape):
        return jax.random.normal(self._next(), shape, dtype=jnp.bfloat16)

    def randint(self, lo, hi, shape):
        return jax.random.randint(self._next(), shape, lo, hi, dtype=jnp.int32)

    def uniform(self, shape, lo=0.0, hi=1.0):
        return jax.random.uniform(self._next(), shape, jnp.bfloat16, lo, hi)

    def permutation(self, n):
        return jax.random.permutation(self._next(), n)
kernel_name = 'adaLN_cond__sliding_block_cached__mixer_s_mlp__decode'

def setup_inputs():
    _rng = _Rng(jax.random.key(int.from_bytes(__import__("os").urandom(4), "little")))
    _w = lambda a: (lambda t: t.astype(jnp.bfloat16) if jnp.issubdtype(t.dtype, jnp.floating) else t)(jnp.asarray(a))

    def _A_setup():
        B, Sq, D = (1, 1, 448)
        Hq, Hkv, Sk, Dh = (16, 8, 65536, 256)
        assert Hq % Hkv == 0, (Hq, Hkv)
        return {'x': _w((lambda *s: _rng.normal(s) * 0.05)(B, Sq, D)), 'k_cache': _w((lambda *s: _rng.normal(s) * 0.05)(B, Hkv, Sk, Dh)), 'v_cache': _w((lambda *s: _rng.normal(s) * 0.05)(B, Hkv, Sk, Dh)), 'wq': _w((lambda *s: _rng.normal(s) * 0.05)(D, Hq * Dh) * D ** (-0.5)), 'wo': _w((lambda *s: _rng.normal(s) * 0.05)(Hq * Dh, D) * (Hq * Dh) ** (-0.5))}
    _A_in = _A_setup()

    def _B_setup():
        B, S, D, F = (1, 1, 448, 1792)
        return {'x': _w((lambda *s: _rng.normal(s) * 0.05)(B, S, D)), 'w1': _w((lambda *s: _rng.normal(s) * 0.05)(D, D) * D ** (-0.5)), 'w2': _w((lambda *s: _rng.normal(s) * 0.05)(D, D) * D ** (-0.5)), 'w3': _w((lambda *s: _rng.normal(s) * 0.05)(D, F) * D ** (-0.5)), 'w4': _w((lambda *s: _rng.normal(s) * 0.05)(F, D) * F ** (-0.5))}
    _B_in = _B_setup()
    return {'A_x': _A_in['x'], 'A_k_cache': _A_in['k_cache'], 'A_v_cache': _A_in['v_cache'], 'A_wq': _A_in['wq'], 'A_wo': _A_in['wo'], 'B_x': _B_in['x'], 'B_w1': _B_in['w1'], 'B_w2': _B_in['w2'], 'B_w3': _B_in['w3'], 'B_w4': _B_in['w4'], 'c': _w((lambda *s: _rng.normal(s) * 0.05)(1, 448)), 'w_mod': _w((lambda *s: _rng.normal(s) * 0.05)(448, 6 * 448) * 448 ** (-0.5))}

def reference(A_x, A_k_cache, A_v_cache, A_wq, A_wo, B_x, B_w1, B_w2, B_w3, B_w4, c, w_mod):

    def _A_ref(x, k_cache, v_cache, wq, wo):
        B, Sq, D = x.shape
        Hq, Dh = (16, 256)
        Hkv, Sk = (k_cache.shape[1], k_cache.shape[2])
        W = min(4096, max(256, Sk // 4))
        rep = Hq // Hkv
        q = (lambda x, *d: x.transpose(*d))((x @ wq).reshape(B, Sq, Hq, Dh), 0, 2, 1, 3)
        k = jnp.repeat(k_cache[:, :, Sk - W:, :], rep, axis=1)
        v = jnp.repeat(v_cache[:, :, Sk - W:, :], rep, axis=1)
        scores = jnp.einsum('bhqd,bhkd->bhqk', q, k) * Dh ** (-0.5)
        p = _softmax(scores, axis=-1)
        o = jnp.einsum('bhqk,bhkd->bhqd', p, v)
        return (lambda x, *d: x.transpose(*d))(o, 0, 2, 1, 3).reshape(B, Sq, Hq * Dh) @ wo

    def _B_ref(x, w1, w2, w3, w4):
        B, S, D = x.shape
        h = _gelu(_layernorm(x, axis=-1) @ w1)
        c = D // 4
        g0 = jnp.pad(h[:, :, 0 * c:1 * c], ((0, 0), (1, 0), (0, 0)))[:, :S, :]
        g1 = jnp.pad(h[:, :, 1 * c:2 * c], ((0, 0), (0, 1), (0, 0)))[:, 1:, :]
        g2 = jnp.pad(h[:, :, 2 * c:3 * c], ((0, 0), (2, 0), (0, 0)))[:, :S, :]
        g3 = jnp.pad(h[:, :, 3 * c:], ((0, 0), (0, 2), (0, 0)))[:, 2:, :]
        hs = jnp.concatenate([g0, g1, g2, g3], axis=-1) @ w2
        x1 = x + hs
        h2 = _gelu(_layernorm(x1, axis=-1) @ w3) @ w4
        return x1 + h2
    x = A_x
    mod = (_silu(c) @ w_mod).reshape(c.shape[0], 6, 1, -1)
    sa, ca, ga, sb, cb, gb = (mod[:, 0].copy(), mod[:, 1].copy(), mod[:, 2].copy(), mod[:, 3].copy(), mod[:, 4].copy(), mod[:, 5].copy())
    h = _layernorm(x, axis=-1) * (1 + ca) + sa
    x = x + ga * _A_ref(h, A_k_cache, A_v_cache, A_wq, A_wo)
    h = _layernorm(x, axis=-1) * (1 + cb) + sb
    x = x + gb * _B_ref(h, B_w1, B_w2, B_w3, B_w4)
    return x
```

```python
import jax
import jax.numpy as jnp
from jax import lax
from jax.experimental import pallas as pl
from jax.experimental.pallas import tpu as pltpu

D, F = 448, 1792
HQ, HKV, DH = 16, 8, 256
WINDOW = 4096
EPS = 1e-5
ROWS = 8
PIECE = 32
BLOCK = 256
BLOCKS = WINDOW // BLOCK
LAG = 4
HEADS = (1, 0, 3, 7, 4, 6, 5, 2)
M_A, M_KV, M_T = 4, 4, 4
W4_GROUPS = ((0, 32), (32, 16), (48, 8))
W4_ORDER = [r + s for r in range(8) for s in (0, 8, 16, 24)] + [r + s for r in range(8) for s in (32, 40)] + list(range(48, 56))
W4_FAST = 32
SKIP = ()
BF16, F32 = jnp.bfloat16, jnp.float32

RING = LAG + 1
S_XC, S_WM, S_WQ, S_WO, S_W3, S_KV = range(6)
S_W4 = S_KV + RING


def _layernorm(x):
    d = x - jnp.sum(x, axis=-1, keepdims=True) * (1.0 / D)
    return d * lax.rsqrt(jnp.sum(d * d, axis=-1, keepdims=True) * (1.0 / D) + EPS)


def _dot(a, b):
    return lax.dot_general(a, b, (((1,), (0,)), ((), ())), preferred_element_type=F32)


def _dot_t(a, b):
    return lax.dot_general(a, b, (((1,), (1,)), ((), ())), preferred_element_type=F32)


def _ds(start, size, align=None):
    return pl.ds(start if isinstance(start, int) else pl.multiple_of(start, align or size), size)


def _loop(lo, hi, body):
    lax.fori_loop(lo, hi, lambda i, carry: body(i), None)


def _kernel(x_hbm, c_hbm, wm_hbm, wq_hbm, k_hbm, v_hbm, wo_hbm, w3_hbm, w4_hbm, out_hbm,
            x_ref, c_ref, wm_ref, wq_ref, k_ref, v_ref, wo_ref, w3_ref, w4_ref,
            mod_ref, q_ref, s_ref, max_ref, sum_ref, ctx_ref, acc_ref, out_ref, sems):
    first_key = k_hbm.shape[2] - WINDOW

    def tiles(hbm, ref, sem, row, col, cols, rows=1):
        at = (_ds(row * 8, rows * 8, 8), _ds(col * 128, cols * 128, 128))
        return pltpu.make_async_copy(hbm.at[at], ref.at[at], sems.at[sem])

    def enqueue(copies, every):
        for i, copy in enumerate(copies):
            copy.start(priority=int(i % every != every - 1))

    def landed(ref, sem):
        pltpu.make_async_copy(ref, ref, sems.at[sem]).wait()

    def wide(hbm, ref, sem, i):
        return [tiles(hbm, ref, sem, row + (i >> 2), (i & 3) * 8, 8) for row in range(0, 56, 8)]

    def narrow(hbm, ref, sem, col, i):
        enqueue([tiles(hbm, ref, sem, row + (i >> 1), col + (i & 1) * 7, 7) for row in range(0, 56, 14)], M_T)

    def cache_block(hbm, ref, b, sem):
        start = first_key + (b >> 3) * 2048 + (b & 7) * (BLOCK // 2)

        def body(i):
            enqueue([pltpu.make_async_copy(hbm.at[0, h, _ds(start + s * 1024 + i * PIECE, PIECE)],
                                           ref.at[b, h, _ds(s * (BLOCK // 2) + i * PIECE, PIECE)], sems.at[sem])
                     for s in range(2) for h in HEADS], M_KV)
        _loop(0, BLOCK // 2 // PIECE, body)

    even = (lax.broadcasted_iota(jnp.int32, (ROWS, DH), 0) & 1) == 0
    small = [pltpu.make_async_copy(c_hbm, c_ref, sems.at[S_XC]), pltpu.make_async_copy(x_hbm, x_ref, sems.at[S_XC])]

    def condition(t):
        c = jnp.broadcast_to(c_ref[...].astype(F32), (ROWS, D))
        both = _dot((c * jax.nn.sigmoid(c)).astype(BF16), wm_ref[:, _ds(t * 2 * D, 2 * D)])
        mod_ref[2 * t] = both[:, :D]
        mod_ref[2 * t + 1] = both[:, D:]

    def condition_attention():
        for copy in small:
            copy.wait()
        landed(wm_ref.at[:, :2 * D], S_WM)
        condition(0)

    def queries():
        landed(wq_ref, S_WQ)
        x = jnp.broadcast_to(x_ref[0].astype(F32), (ROWS, D))
        h_in = (_layernorm(x) * (1.0 + mod_ref[1]) + mod_ref[0]).astype(BF16)

        def body(h):
            q = _dot(h_in, wq_ref[:, _ds(h * 2 * DH, 2 * DH)]) * DH ** -0.5
            q_ref[h] = jnp.where(even, q[:, :DH], q[:, DH:])
            max_ref[h] = jnp.full((ROWS, 128), -jnp.inf, F32)
            sum_ref[h] = jnp.zeros((ROWS, 128), F32)
            ctx_ref[h] = jnp.zeros((ROWS, DH), F32)
        _loop(0, HKV, body)

    def scores(b):
        for h in range(HKV):
            s = _dot_t(q_ref[h].astype(BF16), k_ref[b, h])
            s_ref[b, h] = s
            max_ref[h] = jnp.maximum(max_ref[h], jnp.maximum(s[:, :128], s[:, 128:]))

    def row_maxima():
        for h in range(HKV):
            max_ref[h] = jnp.broadcast_to(jnp.max(max_ref[h], axis=-1, keepdims=True), (ROWS, 128))

    def context(b):
        for h in range(HKV):
            p = jnp.exp(s_ref[b, h] - jnp.concatenate([max_ref[h]] * 2, axis=1))
            sum_ref[h] += p[:, :128] + p[:, 128:]
            ctx_ref[h] += _dot(p.astype(BF16), v_ref[b, h])

    def normalize():
        for h in range(HKV):
            ctx_ref[h] = ctx_ref[h] / jnp.sum(sum_ref[h], axis=-1, keepdims=True)
        acc_ref[...] = jnp.zeros((ROWS, D), F32)

    def project(h):
        o = ctx_ref[h]
        o = jnp.concatenate([jnp.where(even, o, 0.0), jnp.where(even, 0.0, o)], axis=1).astype(BF16)
        return _dot_t(o, wo_ref[:, _ds(h * 2 * DH, 2 * DH)])

    def head(i):
        enqueue(wide(wq_hbm, wq_ref, S_WQ, i) + wide(wo_hbm, wo_ref, S_WO, i), M_A)
        pl.when(i < 28)(lambda: enqueue([tiles(wm_hbm, wm_ref, S_WM, row + i, 0, 7) for row in (0, 28)], 2))
    _loop(0, 32, head)
    enqueue(small, 2)

    def step(t, slot):
        done = jnp.where(slot == RING - 1, 0, slot + 1)
        pl.when(t < BLOCKS)(lambda: cache_block(k_hbm, k_ref, t, S_KV + slot))
        pl.when((t >= BLOCKS) & (t < 2 * BLOCKS))(lambda: cache_block(v_hbm, v_ref, t - BLOCKS, S_KV + slot))
        pl.when(t >= 2 * BLOCKS)(lambda: _loop((t - 2 * BLOCKS) * 28 // LAG, (t - 2 * BLOCKS + 1) * 28 // LAG,
                                               lambda i: narrow(wm_hbm, wm_ref, S_WM, 7, i)))
        pl.when(t == LAG - 2)(condition_attention)
        pl.when(t == LAG - 1)(queries)

        @pl.when((t >= LAG) & (t < BLOCKS + LAG))
        def _():
            landed(k_ref.at[t - LAG], S_KV + done)
            if 'scores' not in SKIP: scores(t - LAG)

        pl.when(t == BLOCKS + LAG)(row_maxima)

        @pl.when(t >= BLOCKS + LAG)
        def _():
            landed(v_ref.at[t - BLOCKS - LAG], S_KV + done)
            if 'context' not in SKIP: context(t - BLOCKS - LAG)
        return done

    lax.fori_loop(0, 2 * BLOCKS + LAG, step, 0)
    landed(wo_ref, S_WO)
    normalize()

    def output(h):
        _loop(h * 7 >> 1, (h + 1) * 7 >> 1, lambda i: narrow(w3_hbm, w3_ref, S_W3, 0, i))
        if 'project' not in SKIP: acc_ref[...] += project(h)
    _loop(0, HKV, output)
    landed(wm_ref.at[:, 2 * D:], S_WM)

    def condition_mlp(t):
        _loop(7 * t - 7, 7 * t, lambda i: enqueue([tiles(w4_hbm, w4_ref, S_W4, row + i, 0, 7) for row in range(0, 56, 14)], M_T))
        condition(t)
    _loop(1, 3, condition_mlp)
    last = [tiles(w4_hbm, w4_ref, S_W4 + sum(row >= g[0] for g in W4_GROUPS), row, 7, 7) for row in W4_ORDER]
    enqueue(last[:W4_FAST], M_T)
    enqueue(last[W4_FAST:], 99)
    attn = acc_ref[...]
    x = jnp.broadcast_to(x_ref[0].astype(F32), (ROWS, D))
    x = x + mod_ref[2] * (attn + pltpu.roll(attn, 1, 0))
    h_mlp = _layernorm(x) * (1.0 + mod_ref[4]) + mod_ref[3]
    normed = _layernorm(h_mlp).astype(BF16)
    y = h_mlp

    landed(w3_ref, S_W3)
    hidden = jax.nn.gelu(_dot(normed, w3_ref[...]), approximate=True).astype(BF16)
    landed(w4_ref.at[:, :F // 2], S_W4)
    gate = mod_ref[5]
    acc_ref[...] = x + gate * (y + _dot_t(hidden[:, :F // 2], w4_ref[:, :F // 2]))
    for g, (row, rows) in enumerate(W4_GROUPS):
        at = pl.ds(row * 8, rows * 8)
        landed(w4_ref.at[at, F // 2:], S_W4 + 1 + g)
        y = acc_ref[:, at]
        if 'w4' not in SKIP: y = y + mod_ref[5, :, at] * _dot_t(hidden[:, F // 2:], w4_ref[at, F // 2:])
        out_ref[0, :, at] = y[0:1].astype(BF16)
    store = pltpu.make_async_copy(out_ref, out_hbm, sems.at[S_XC])
    store.start()
    store.wait()


@jax.jit
def pallas_adaLN_cond__sliding_block_cached__mixer_s_mlp__decode_kernel(
    A_x: jax.Array,
    A_k_cache: jax.Array,
    A_v_cache: jax.Array,
    A_wq: jax.Array,
    A_wo: jax.Array,
    B_x: jax.Array,
    B_w1: jax.Array,
    B_w2: jax.Array,
    B_w3: jax.Array,
    B_w4: jax.Array,
    c: jax.Array,
    w_mod: jax.Array,
):
    keys = A_k_cache.shape[2]
    assert A_x.shape == (1, 1, D) and A_k_cache.shape == (1, HKV, keys, DH)
    assert min(4096, max(256, keys // 4)) == WINDOW and keys % PIECE == 0
    hbm = pl.BlockSpec(memory_space=pltpu.HBM)
    return pl.pallas_call(
        _kernel,
        out_shape=jax.ShapeDtypeStruct(A_x.shape, A_x.dtype),
        in_specs=[hbm] * 9,
        out_specs=hbm,
        scratch_shapes=[
            pltpu.VMEM((1, 1, D), BF16),
            pltpu.VMEM((1, D), BF16),
            pltpu.VMEM((D, 6 * D), BF16),
            pltpu.VMEM((D, HQ * DH), BF16),
            pltpu.VMEM((BLOCKS, HKV, BLOCK, DH), BF16),
            pltpu.VMEM((BLOCKS, HKV, BLOCK, DH), BF16),
            pltpu.VMEM((D, HQ * DH), BF16),
            pltpu.VMEM((D, F), BF16),
            pltpu.VMEM((D, F), BF16),
            pltpu.VMEM((6, ROWS, D), F32),
            pltpu.VMEM((HKV, ROWS, DH), F32),
            pltpu.VMEM((BLOCKS, HKV, ROWS, BLOCK), F32),
            pltpu.VMEM((HKV, ROWS, 128), F32),
            pltpu.VMEM((HKV, ROWS, 128), F32),
            pltpu.VMEM((HKV, ROWS, DH), F32),
            pltpu.VMEM((ROWS, D), F32),
            pltpu.VMEM((1, 1, D), BF16),
            pltpu.SemaphoreType.DMA((S_W4 + 1 + len(W4_GROUPS),)),
        ],
        compiler_params=pltpu.CompilerParams(
            vmem_limit_bytes=100 * 2**20,
            disable_bounds_checks=True,
            disable_semaphore_checks=True,
        ),
        name="adaln_decode",
    )(A_x, c, w_mod, A_wq, A_k_cache, A_v_cache, A_wo.T, B_w3, B_w4.T)
```

```python
import jax
import jax.numpy as jnp
from jax import lax
from jax.experimental import pallas as pl
from jax.experimental.pallas import tpu as pltpu

D, F = 448, 1792
HQ, HKV, DH = 16, 8, 256
WINDOW = 4096
EPS = 1e-5
ROWS = 8
PIECE = 32
BLOCK = 256
BLOCKS = WINDOW // BLOCK
LAG = 4
HEADS = (1, 0, 3, 7, 4, 6, 5, 2)
M_A, M_KV, M_T = 4, 4, 4
W4_GROUPS = ((0, 32), (32, 16), (48, 8))
W4_ORDER = [r + s for r in range(8) for s in (0, 8, 16, 24)] + [r + s for r in range(8) for s in (32, 40)] + list(range(48, 56))
EARLY_MOD, LATE_MOD = 18 * 128, 3 * 128
GATE_GROUPS = (0, 4, 6, 7)
WM_RUNS = ((7, 6), (13, 5))
SPLIT = (12, 32, 56, 84)
SKIP = ()
BF16, F32 = jnp.bfloat16, jnp.float32

RING = LAG + 1
S_XC, S_WM, S_WQ, S_WO, S_W3, S_KV = range(6)
S_GATE = S_KV + RING
S_W4 = S_GATE + 4


def _layernorm(x):
    d = x - jnp.sum(x, axis=-1, keepdims=True) * (1.0 / D)
    return d * lax.rsqrt(jnp.sum(d * d, axis=-1, keepdims=True) * (1.0 / D) + EPS)


def _dot(a, b):
    return lax.dot_general(a, b, (((1,), (0,)), ((), ())), preferred_element_type=F32)


def _dot_t(a, b):
    return lax.dot_general(a, b, (((1,), (1,)), ((), ())), preferred_element_type=F32)


def _ds(start, size, align=None):
    return pl.ds(start if isinstance(start, int) else pl.multiple_of(start, align or size), size)


def _loop(lo, hi, body):
    lax.fori_loop(lo, hi, lambda i, carry: body(i), None)


def _kernel(x_hbm, c_hbm, wm_hbm, wq_hbm, k_hbm, v_hbm, wo_hbm, w3_hbm, w4_hbm, out_hbm,
            x_ref, c_ref, wm_ref, wq_ref, k_ref, v_ref, wo_ref, w3_ref, w4_ref,
            mod_ref, wg_ref, col_ref, q_ref, s_ref, max_ref, sum_ref, ctx_ref, acc_ref, hid_ref, out_ref, sems):
    first_key = k_hbm.shape[2] - WINDOW

    def tiles(hbm, ref, sem, row, col, cols, rows=1):
        at = (_ds(row * 8, rows * 8, 8), _ds(col * 128, cols * 128, 128))
        return pltpu.make_async_copy(hbm.at[at], ref.at[at], sems.at[sem])

    def enqueue(copies, every):
        for i, copy in enumerate(copies):
            copy.start(priority=int(i % every != every - 1))

    def landed(ref, sem):
        pltpu.make_async_copy(ref, ref, sems.at[sem]).wait()

    def wide(hbm, ref, sem, i):
        return [tiles(hbm, ref, sem, row + (i >> 2), (i & 3) * 8, 8) for row in range(0, 56, 8)]

    def narrow(hbm, ref, sem, i, *runs):
        for col, cols in runs:
            enqueue([tiles(hbm, ref, sem, row + i, col, cols) for row in range(0, 56, 14)], M_T)

    def gate_weights(i):
        sem = S_GATE + sum(i >= g for g in GATE_GROUPS[1:-1])
        return [pltpu.make_async_copy(wm_hbm.at[pl.ds(112 * s + 16 * i, 16), pl.ds(EARLY_MOD, LATE_MOD)],
                                      wg_ref.at[i, pl.ds(16 * s, 16)], sems.at[sem]) for s in range(4)]

    def cache_block(hbm, ref, b, sem):
        start = first_key + (b >> 3) * 2048 + (b & 7) * (BLOCK // 2)

        def body(i):
            enqueue([pltpu.make_async_copy(hbm.at[0, h, _ds(start + s * 1024 + i * PIECE, PIECE)],
                                           ref.at[b, h, _ds(s * (BLOCK // 2) + i * PIECE, PIECE)], sems.at[sem])
                     for s in range(2) for h in HEADS], M_KV)
        _loop(0, BLOCK // 2 // PIECE, body)

    even = (lax.broadcasted_iota(jnp.int32, (ROWS, DH), 0) & 1) == 0
    small = [pltpu.make_async_copy(c_hbm, c_ref, sems.at[S_XC]), pltpu.make_async_copy(x_hbm, x_ref, sems.at[S_XC])]

    def silu_c():
        c = jnp.broadcast_to(c_ref[...].astype(F32), (ROWS, D))
        return (c * jax.nn.sigmoid(c)).astype(BF16)

    def condition(t):
        both = _dot(silu_c(), wm_ref[:, t * 2 * D:(t + 1) * 2 * D])
        mod_ref[2 * t] = both[:, :D]
        mod_ref[2 * t + 1] = both[:, D:]

    def condition_attention():
        for copy in small:
            copy.wait()
        landed(wm_ref.at[:, :2 * D], S_WM)
        condition(0)
        x = jnp.broadcast_to(x_ref[0].astype(F32), (ROWS, D))
        acc_ref[...] = _layernorm(x) * (1.0 + mod_ref[1]) + mod_ref[0]

    def queries(part):
        h_in = acc_ref[...].astype(BF16)

        def body(h):
            q = _dot(h_in, wq_ref[:, _ds(h * 2 * DH, 2 * DH)]) * DH ** -0.5
            q_ref[h] = jnp.where(even, q[:, :DH], q[:, DH:])
            max_ref[h] = jnp.full((ROWS, 128), -jnp.inf, F32)
            sum_ref[h] = jnp.zeros((ROWS, 128), F32)
            ctx_ref[h] = jnp.zeros((ROWS, DH), F32)
        _loop(3 * part, jnp.minimum(3 * part + 3, HKV), body)

    def scores(b):
        for h in range(HKV):
            s = _dot_t(q_ref[h].astype(BF16), k_ref[b, h])
            s_ref[b, h] = s
            max_ref[h] = jnp.maximum(max_ref[h], jnp.maximum(s[:, :128], s[:, 128:]))

    def row_maxima():
        for h in range(HKV):
            max_ref[h] = jnp.broadcast_to(jnp.max(max_ref[h], axis=-1, keepdims=True), (ROWS, 128))

    def context(b):
        for h in range(HKV):
            p = jnp.exp(s_ref[b, h] - jnp.concatenate([max_ref[h]] * 2, axis=1))
            sum_ref[h] += p[:, :128] + p[:, 128:]
            ctx_ref[h] += _dot(p.astype(BF16), v_ref[b, h])

    def normalize():
        for h in range(HKV):
            ctx_ref[h] = ctx_ref[h] / jnp.sum(sum_ref[h], axis=-1, keepdims=True)
        acc_ref[...] = jnp.zeros((ROWS, D), F32)

    def project(h):
        o = ctx_ref[h]
        o = jnp.concatenate([jnp.where(even, o, 0.0), jnp.where(even, 0.0, o)], axis=1).astype(BF16)
        return _dot_t(o, wo_ref[:, _ds(h * 2 * DH, 2 * DH)])

    def head(i):
        enqueue(wide(wq_hbm, wq_ref, S_WQ, i) + wide(wo_hbm, wo_ref, S_WO, i), M_A)
        pl.when(i < 28)(lambda: enqueue([tiles(wm_hbm, wm_ref, S_WM, row + i, 0, 7) for row in (0, 28)], 2))
        pl.when(i == 8)(lambda: enqueue(small, 2))
    _loop(0, 32, head)

    def step(t, slot):
        done = jnp.where(slot == RING - 1, 0, slot + 1)
        pl.when(t < BLOCKS)(lambda: cache_block(k_hbm, k_ref, t, S_KV + slot))
        pl.when((t >= BLOCKS) & (t < 2 * BLOCKS))(lambda: cache_block(v_hbm, v_ref, t - BLOCKS, S_KV + slot))
        pl.when(t >= 2 * BLOCKS)(lambda: _loop((t - 2 * BLOCKS) * 7 >> 1, (t - 2 * BLOCKS + 1) * 7 >> 1,
                                               lambda i: narrow(wm_hbm, wm_ref, S_WM, i, *WM_RUNS)))
        pl.when(t == 0)(condition_attention)
        pl.when(t == 1)(lambda: landed(wq_ref, S_WQ))
        pl.when((t >= 1) & (t < LAG))(lambda: queries(t - 1))

        @pl.when((t >= LAG) & (t < BLOCKS + LAG))
        def _():
            landed(k_ref.at[t - LAG], S_KV + done)
            if 'scores' not in SKIP: scores(t - LAG)

        pl.when(t == BLOCKS + LAG)(row_maxima)

        @pl.when(t >= BLOCKS + LAG)
        def _():
            landed(v_ref.at[t - BLOCKS - LAG], S_KV + done)
            if 'context' not in SKIP: context(t - BLOCKS - LAG)
        return done

    lax.fori_loop(0, 2 * BLOCKS + LAG, step, 0)
    landed(wo_ref, S_WO)
    normalize()

    def output(h):
        _loop(h * 7 >> 2, (h + 1) * 7 >> 2, lambda i: narrow(w3_hbm, w3_ref, S_W3, i, (0, 7), (7, 7)))
        if 'project' not in SKIP: acc_ref[...] += project(h)
    _loop(0, HKV, output)
    landed(wm_ref.at[:, 2 * D:], S_WM)

    _loop(0, 7, lambda i: narrow(w4_hbm, w4_ref, S_W4, i, (0, 7)))
    condition(1)
    _loop(7, 14, lambda i: narrow(w4_hbm, w4_ref, S_W4, i, (0, 7)))
    c = silu_c()
    rest = _dot(c, wm_ref[:, 4 * D:])
    c = jnp.concatenate([c.astype(F32), jnp.zeros((ROWS, 512 - D), F32)], axis=1)
    for j in range(4):
        col_ref[pl.ds(j * 128, 128)] = jnp.broadcast_to(c[:1, j * 128:(j + 1) * 128], (128, 128)).T
    last = [tiles(w4_hbm, w4_ref, S_W4 + sum(row >= g[0] for g in W4_GROUPS), row, 7, 7) for row in W4_ORDER]
    last += [copy for i in range(7) for copy in gate_weights(i)]
    enqueue(last[:SPLIT[0]], M_T)
    attn = acc_ref[...]
    x = jnp.broadcast_to(x_ref[0].astype(F32), (ROWS, D))
    x = x + mod_ref[2] * (attn + pltpu.roll(attn, 1, 0))
    h_mlp = _layernorm(x) * (1.0 + rest[:, :D]) + mod_ref[3]
    acc_ref[...] = _layernorm(h_mlp)
    enqueue(last[SPLIT[0]:SPLIT[1]], M_T)
    landed(w3_ref, S_W3)
    hid_ref[...] = jax.nn.gelu(_dot(acc_ref[...].astype(BF16), w3_ref[...]), approximate=True)
    enqueue(last[SPLIT[1]:SPLIT[2]], M_T)
    enqueue(last[SPLIT[2]:SPLIT[3]], 99)
    landed(w4_ref.at[:, :F // 2], S_W4)
    acc_ref[...] = h_mlp + _dot_t(hid_ref[:, :F // 2].astype(BF16), w4_ref[:, :F // 2])
    enqueue(last[SPLIT[3]:], 99)
    for g, (row, rows) in enumerate(W4_GROUPS):
        at = pl.ds(row * 8, rows * 8)
        landed(w4_ref.at[at, F // 2:], S_W4 + 1 + g)
        acc_ref[:, at] += _dot_t(hid_ref[:, F // 2:].astype(BF16), w4_ref[at, F // 2:])
    gate = [jnp.zeros((ROWS, 128), F32)] * 3
    for g, (lo, hi) in enumerate(zip(GATE_GROUPS[:-1], GATE_GROUPS[1:])):
        landed(wg_ref.at[pl.ds(lo, hi - lo)], S_GATE + g)
        for i in range(lo, hi):
            for s in range(4):
                col = col_ref[pl.ds(112 * s + 16 * i, 16)]
                for j in range(3):
                    prod = wg_ref[i, pl.ds(16 * s, 16), pl.ds(j * 128, 128)].astype(F32) * col
                    gate[j] = gate[j] + (prod[:8] + prod[8:])
    gate = jnp.concatenate([rest[:1, D:]] + [jnp.sum(part, axis=0, keepdims=True) for part in gate], axis=1)
    if 'gate' in SKIP: gate = 1.0
    out_ref[0] = (x[:1] + gate * acc_ref[:1]).astype(BF16)
    store = pltpu.make_async_copy(out_ref, out_hbm, sems.at[S_XC])
    store.start()
    store.wait()


@jax.jit
def pallas_adaLN_cond__sliding_block_cached__mixer_s_mlp__decode_kernel(
    A_x: jax.Array,
    A_k_cache: jax.Array,
    A_v_cache: jax.Array,
    A_wq: jax.Array,
    A_wo: jax.Array,
    B_x: jax.Array,
    B_w1: jax.Array,
    B_w2: jax.Array,
    B_w3: jax.Array,
    B_w4: jax.Array,
    c: jax.Array,
    w_mod: jax.Array,
):
    keys = A_k_cache.shape[2]
    assert A_x.shape == (1, 1, D) and A_k_cache.shape == (1, HKV, keys, DH)
    assert min(4096, max(256, keys // 4)) == WINDOW and keys % PIECE == 0
    hbm = pl.BlockSpec(memory_space=pltpu.HBM)
    return pl.pallas_call(
        _kernel,
        out_shape=jax.ShapeDtypeStruct(A_x.shape, A_x.dtype),
        in_specs=[hbm] * 9,
        out_specs=hbm,
        scratch_shapes=[
            pltpu.VMEM((1, 1, D), BF16),
            pltpu.VMEM((1, D), BF16),
            pltpu.VMEM((D, EARLY_MOD), BF16),
            pltpu.VMEM((D, HQ * DH), BF16),
            pltpu.VMEM((BLOCKS, HKV, BLOCK, DH), BF16),
            pltpu.VMEM((BLOCKS, HKV, BLOCK, DH), BF16),
            pltpu.VMEM((D, HQ * DH), BF16),
            pltpu.VMEM((D, F), BF16),
            pltpu.VMEM((D, F), BF16),
            pltpu.VMEM((6, ROWS, D), F32),
            pltpu.VMEM((7, 64, LATE_MOD), BF16),
            pltpu.VMEM((512, 128), F32),
            pltpu.VMEM((HKV, ROWS, DH), F32),
            pltpu.VMEM((BLOCKS, HKV, ROWS, BLOCK), F32),
            pltpu.VMEM((HKV, ROWS, 128), F32),
            pltpu.VMEM((HKV, ROWS, 128), F32),
            pltpu.VMEM((HKV, ROWS, DH), F32),
            pltpu.VMEM((ROWS, D), F32),
            pltpu.VMEM((ROWS, F), F32),
            pltpu.VMEM((1, 1, D), BF16),
            pltpu.SemaphoreType.DMA((S_W4 + 1 + len(W4_GROUPS),)),
        ],
        compiler_params=pltpu.CompilerParams(
            vmem_limit_bytes=100 * 2**20,
            disable_bounds_checks=True,
            disable_semaphore_checks=True,
        ),
        name="adaln_decode",
    )(A_x, c, w_mod, A_wq, A_k_cache, A_v_cache, A_wo.T, B_w3, B_w4.T)
```

```python
import jax
import jax.numpy as jnp
from jax import lax
from jax.experimental import pallas as pl
from jax.experimental.pallas import tpu as pltpu

D, F = 448, 1792
HQ, HKV, DH = 16, 8, 256
WINDOW = 4096
EPS = 1e-5
ROWS = 8
PIECE = 32
BLOCK = 256
BLOCKS = WINDOW // BLOCK
LAG = 4
HEADS = (1, 4, 7, 3, 2, 0, 5, 6)
M_A, M_KV, M_T = 4, 4, 4
W4_GROUPS = ((0, 32), (32, 16), (48, 8))
W4_ORDER = [r + s for r in range(8) for s in (0, 8, 16, 24)] + [r + s for r in range(8) for s in (32, 40)] + list(range(48, 56))
EARLY_MOD, LATE_MOD = 18 * 128, 3 * 128
GATE_ROWS = 16
GATE_ORDER = [i + 6 * s for i in range(6) for s in range(3)] + list(range(18, 28))
GATE_GROUPS = (0, 16, 24, 28)
WM_RUNS = ((7, 6), (13, 5))
W4_FIRST = [54, 55] + [r + s for r in range(12, 18) for s in (0, 18, 36)]
MIX = 0
M_6 = 6
SPLIT = (12, 32, 56, 84)
SKIP = ()
BF16, F32 = jnp.bfloat16, jnp.float32

RING = LAG + 1
S_XC, S_WM, S_WQ, S_WO, S_W3, S_KV = range(6)
S_GATE = S_KV + RING
S_W4 = S_GATE + 4


def _layernorm(x):
    d = x - jnp.sum(x, axis=-1, keepdims=True) * (1.0 / D)
    return d * lax.rsqrt(jnp.sum(d * d, axis=-1, keepdims=True) * (1.0 / D) + EPS)


def _dot(a, b):
    return lax.dot_general(a, b, (((1,), (0,)), ((), ())), preferred_element_type=F32)


def _dot_t(a, b):
    return lax.dot_general(a, b, (((1,), (1,)), ((), ())), preferred_element_type=F32)


def _ds(start, size, align=None):
    return pl.ds(start if isinstance(start, int) else pl.multiple_of(start, align or size), size)


def _loop(lo, hi, body):
    lax.fori_loop(lo, hi, lambda i, carry: body(i), None)


def _kernel(x_hbm, c_hbm, wm_hbm, wq_hbm, k_hbm, v_hbm, wo_hbm, w3_hbm, w4_hbm, out_hbm,
            x_ref, c_ref, wm_ref, wq_ref, k_ref, v_ref, wo_ref, w3_ref, w4_ref,
            mod_ref, wg_ref, col_ref, q_ref, s_ref, max_ref, sum_ref, ctx_ref, acc_ref, hid_ref, out_ref, sems):
    first_key = k_hbm.shape[2] - WINDOW

    def tiles(hbm, ref, sem, row, col, cols, rows=1):
        at = (_ds(row * 8, rows * 8, 8), _ds(col * 128, cols * 128, 128))
        return pltpu.make_async_copy(hbm.at[at], ref.at[at], sems.at[sem])

    def enqueue(copies, every):
        for i, copy in enumerate(copies):
            copy.start(priority=int(i % every != every - 1))

    def landed(ref, sem):
        pltpu.make_async_copy(ref, ref, sems.at[sem]).wait()

    def wide(hbm, ref, sem, i):
        return [tiles(hbm, ref, sem, row + (i >> 2), (i & 3) * 8, 8) for row in range(0, 56, 8)]

    def w_mod_and_w3(i, rows_m, rows_3):
        for (col, cols), half in zip(WM_RUNS, (0, 7)):
            enqueue([tiles(wm_hbm, wm_ref, S_WM, row + i, col, cols) for row in rows_m]
                    + [tiles(w3_hbm, w3_ref, S_W3, row + i, half, 7) for row in rows_3], M_T)

    def w3_and_w4(i):
        for j in range(2):
            enqueue([tiles(w3_hbm, w3_ref, S_W3, row + 12 + i, 7 * j, 7) for row in (0, 18, 36)]
                    + [tiles(w4_hbm, w4_ref, S_W4, row + 2 * i + j, 0, 7) for row in (0, 18, 36)], M_6)

    def gate_weights(i):
        return pltpu.make_async_copy(wm_hbm.at[pl.ds(GATE_ROWS * GATE_ORDER[i], GATE_ROWS), pl.ds(EARLY_MOD, LATE_MOD)],
                                     wg_ref.at[pl.ds(GATE_ROWS * i, GATE_ROWS)],
                                     sems.at[S_GATE + sum(i >= g for g in GATE_GROUPS[1:-1])])

    def cache_block(hbm, ref, b, sem):
        start = first_key + b * (BLOCK // 2)
        apart = 3072 - (b >> 3) * 2048

        def body(i):
            enqueue([pltpu.make_async_copy(hbm.at[0, h, _ds(start + s * apart + i * PIECE, PIECE)],
                                           ref.at[b, h, _ds(s * (BLOCK // 2) + i * PIECE, PIECE)], sems.at[sem])
                     for s in range(2) for h in HEADS], M_KV)
        _loop(0, BLOCK // 2 // PIECE, body)

    even = (lax.broadcasted_iota(jnp.int32, (ROWS, DH), 0) & 1) == 0
    small = [pltpu.make_async_copy(c_hbm, c_ref, sems.at[S_XC]), pltpu.make_async_copy(x_hbm, x_ref, sems.at[S_XC])]

    def silu_c():
        c = jnp.broadcast_to(c_ref[...].astype(F32), (ROWS, D))
        return (c * jax.nn.sigmoid(c)).astype(BF16)

    def condition(t):
        both = _dot(silu_c(), wm_ref[:, t * 2 * D:(t + 1) * 2 * D])
        mod_ref[2 * t] = both[:, :D]
        mod_ref[2 * t + 1] = both[:, D:]

    def condition_attention():
        for copy in small:
            copy.wait()
        landed(wm_ref.at[:, :2 * D], S_WM)
        condition(0)
        x = jnp.broadcast_to(x_ref[0].astype(F32), (ROWS, D))
        acc_ref[...] = _layernorm(x) * (1.0 + mod_ref[1]) + mod_ref[0]

    def queries(part):
        h_in = acc_ref[...].astype(BF16)

        def body(h):
            q = _dot(h_in, wq_ref[:, _ds(h * 2 * DH, 2 * DH)]) * DH ** -0.5
            q_ref[h] = jnp.where(even, q[:, :DH], q[:, DH:])
            max_ref[h] = jnp.full((ROWS, 128), -jnp.inf, F32)
            sum_ref[h] = jnp.zeros((ROWS, 128), F32)
            ctx_ref[h] = jnp.zeros((ROWS, DH), F32)
        _loop(3 * part, jnp.minimum(3 * part + 3, HKV), body)

    def scores(b):
        for h in range(HKV):
            s = _dot_t(q_ref[h].astype(BF16), k_ref[b, h])
            s_ref[b, h] = s
            max_ref[h] = jnp.maximum(max_ref[h], jnp.maximum(s[:, :128], s[:, 128:]))

    def row_maxima():
        for h in range(HKV):
            max_ref[h] = jnp.broadcast_to(jnp.max(max_ref[h], axis=-1, keepdims=True), (ROWS, 128))

    def context(b):
        for h in range(HKV):
            p = jnp.exp(s_ref[b, h] - jnp.concatenate([max_ref[h]] * 2, axis=1))
            sum_ref[h] += p[:, :128] + p[:, 128:]
            ctx_ref[h] += _dot(p.astype(BF16), v_ref[b, h])

    def normalize():
        for h in range(HKV):
            ctx_ref[h] = ctx_ref[h] / jnp.sum(sum_ref[h], axis=-1, keepdims=True)
        acc_ref[...] = jnp.zeros((ROWS, D), F32)

    def project(h):
        o = ctx_ref[h]
        o = jnp.concatenate([jnp.where(even, o, 0.0), jnp.where(even, 0.0, o)], axis=1).astype(BF16)
        return _dot_t(o, wo_ref[:, _ds(h * 2 * DH, 2 * DH)])

    _loop(0, 14, lambda i: enqueue([tiles(wm_hbm, wm_ref, S_WM, row + i, 0, 7) for row in (0, 14, 28, 42)], 4))
    enqueue(small, 2)
    _loop(0, 32, lambda i: enqueue(wide(wq_hbm, wq_ref, S_WQ, i) + wide(wo_hbm, wo_ref, S_WO, i), M_A))

    def step(t, slot):
        done = jnp.where(slot == RING - 1, 0, slot + 1)
        pl.when(t < BLOCKS)(lambda: cache_block(k_hbm, k_ref, t, S_KV + slot))
        pl.when((t >= BLOCKS) & (t < 2 * BLOCKS))(lambda: cache_block(v_hbm, v_ref, t - BLOCKS, S_KV + slot))
        pl.when(t >= 2 * BLOCKS)(lambda: _loop((t - 2 * BLOCKS) * 2, (t - 2 * BLOCKS + 1) * 2,
                                               lambda i: w_mod_and_w3(i, (0, 12, 24, 36, 48), (0, 18, 36))))
        pl.when(t == 0)(condition_attention)
        pl.when(t == 1)(lambda: landed(wq_ref, S_WQ))
        pl.when((t >= 1) & (t < LAG))(lambda: queries(t - 1))

        @pl.when((t >= LAG) & (t < BLOCKS + LAG))
        def _():
            landed(k_ref.at[t - LAG], S_KV + done)
            if 'scores' not in SKIP: scores(t - LAG)

        pl.when(t == BLOCKS + LAG)(row_maxima)

        @pl.when(t >= BLOCKS + LAG)
        def _():
            landed(v_ref.at[t - BLOCKS - LAG], S_KV + done)
            if 'context' not in SKIP: context(t - BLOCKS - LAG)
        return done

    lax.fori_loop(0, 2 * BLOCKS + LAG, step, 0)
    landed(wo_ref, S_WO)
    normalize()

    def output(h):
        pl.when(h < 2)(lambda: enqueue([tiles(w3_hbm, w3_ref, S_W3, 54 + h, 0, 14)], 2))
        pl.when(h < 4)(lambda: w_mod_and_w3(8 + h, (0, 12, 24, 36), (0, 18, 36)))
        pl.when(h >= 4)(lambda: _loop(((h - 4) * 3) >> 1, ((h - 3) * 3) >> 1, w3_and_w4))
        if 'project' not in SKIP: acc_ref[...] += project(h)
    _loop(0, HKV, output)
    last = [tiles(w4_hbm, w4_ref, S_W4, row, 0, 7) for row in W4_FIRST]
    last += [tiles(w4_hbm, w4_ref, S_W4 + sum(row >= g[0] for g in W4_GROUPS), row, 7, 7) for row in W4_ORDER]
    gates = [gate_weights(i) for i in range(len(GATE_ORDER))]
    last = last[:len(last) - MIX] + [copy for pair in zip(last[len(last) - MIX:], gates) for copy in pair] + gates[MIX:]
    enqueue(last[:20], M_T)
    last = last[20:]
    landed(wm_ref.at[:, 2 * D:], S_WM)
    condition(1)
    c = silu_c()
    rest = _dot(c, wm_ref[:, 4 * D:])
    c = jnp.concatenate([c.astype(F32), jnp.zeros((ROWS, 512 - D), F32)], axis=1)
    for j in range(4):
        col_ref[pl.ds(j * 128, 128)] = jnp.broadcast_to(c[:1, j * 128:(j + 1) * 128], (128, 128)).T
    enqueue(last[:SPLIT[0]], M_T)
    attn = acc_ref[...]
    x = jnp.broadcast_to(x_ref[0].astype(F32), (ROWS, D))
    x = x + mod_ref[2] * (attn + pltpu.roll(attn, 1, 0))
    h_mlp = _layernorm(x) * (1.0 + rest[:, :D]) + mod_ref[3]
    acc_ref[...] = _layernorm(h_mlp)
    enqueue(last[SPLIT[0]:SPLIT[1]], M_T)
    landed(w3_ref, S_W3)
    hid_ref[...] = jax.nn.gelu(_dot(acc_ref[...].astype(BF16), w3_ref[...]), approximate=True)
    enqueue(last[SPLIT[1]:SPLIT[2]], M_T)
    enqueue(last[SPLIT[2]:SPLIT[3]], 99)
    landed(w4_ref.at[:, :F // 2], S_W4)
    acc_ref[...] = h_mlp + _dot_t(hid_ref[:, :F // 2].astype(BF16), w4_ref[:, :F // 2])
    enqueue(last[SPLIT[3]:], 99)
    for g, (row, rows) in enumerate(W4_GROUPS):
        at = pl.ds(row * 8, rows * 8)
        landed(w4_ref.at[at, F // 2:], S_W4 + 1 + g)
        acc_ref[:, at] += _dot_t(hid_ref[:, F // 2:].astype(BF16), w4_ref[at, F // 2:])
    gate = [jnp.zeros((ROWS, 128), F32)] * 3
    for g, (lo, hi) in enumerate(zip(GATE_GROUPS[:-1], GATE_GROUPS[1:])):
        landed(wg_ref.at[pl.ds(lo * GATE_ROWS, (hi - lo) * GATE_ROWS)], S_GATE + g)
        rows = [GATE_ROWS * GATE_ORDER[i] + r for i in range(lo, hi) for r in range(0, GATE_ROWS, 8)]
        for i in range(0, len(rows), 2):
            for j in range(3):
                w = wg_ref[pl.ds(lo * GATE_ROWS + 8 * i, 16), pl.ds(j * 128, 128)].astype(F32)
                gate[j] = gate[j] + (w[:8] * col_ref[pl.ds(rows[i], 8)] + w[8:] * col_ref[pl.ds(rows[i + 1], 8)])
    gate = jnp.concatenate([rest[:1, D:]] + [jnp.sum(part, axis=0, keepdims=True) for part in gate], axis=1)
    if 'gate' in SKIP: gate = 1.0
    out_ref[0] = (x[:1] + gate * acc_ref[:1]).astype(BF16)
    store = pltpu.make_async_copy(out_ref, out_hbm, sems.at[S_XC])
    store.start()
    store.wait()


@jax.jit
def pallas_adaLN_cond__sliding_block_cached__mixer_s_mlp__decode_kernel(
    A_x: jax.Array,
    A_k_cache: jax.Array,
    A_v_cache: jax.Array,
    A_wq: jax.Array,
    A_wo: jax.Array,
    B_x: jax.Array,
    B_w1: jax.Array,
    B_w2: jax.Array,
    B_w3: jax.Array,
    B_w4: jax.Array,
    c: jax.Array,
    w_mod: jax.Array,
):
    keys = A_k_cache.shape[2]
    assert A_x.shape == (1, 1, D) and A_k_cache.shape == (1, HKV, keys, DH)
    assert min(4096, max(256, keys // 4)) == WINDOW and keys % PIECE == 0
    hbm = pl.BlockSpec(memory_space=pltpu.HBM)
    return pl.pallas_call(
        _kernel,
        out_shape=jax.ShapeDtypeStruct(A_x.shape, A_x.dtype),
        in_specs=[hbm] * 9,
        out_specs=hbm,
        scratch_shapes=[
            pltpu.VMEM((1, 1, D), BF16),
            pltpu.VMEM((1, D), BF16),
            pltpu.VMEM((D, EARLY_MOD), BF16),
            pltpu.VMEM((D, HQ * DH), BF16),
            pltpu.VMEM((BLOCKS, HKV, BLOCK, DH), BF16),
            pltpu.VMEM((BLOCKS, HKV, BLOCK, DH), BF16),
            pltpu.VMEM((D, HQ * DH), BF16),
            pltpu.VMEM((D, F), BF16),
            pltpu.VMEM((D, F), BF16),
            pltpu.VMEM((6, ROWS, D), F32),
            pltpu.VMEM((D, LATE_MOD), BF16),
            pltpu.VMEM((512, 128), F32),
            pltpu.VMEM((HKV, ROWS, DH), F32),
            pltpu.VMEM((BLOCKS, HKV, ROWS, BLOCK), F32),
            pltpu.VMEM((HKV, ROWS, 128), F32),
            pltpu.VMEM((HKV, ROWS, 128), F32),
            pltpu.VMEM((HKV, ROWS, DH), F32),
            pltpu.VMEM((ROWS, D), F32),
            pltpu.VMEM((ROWS, F), F32),
            pltpu.VMEM((1, 1, D), BF16),
            pltpu.SemaphoreType.DMA((S_W4 + 1 + len(W4_GROUPS),)),
        ],
        compiler_params=pltpu.CompilerParams(
            vmem_limit_bytes=100 * 2**20,
            disable_bounds_checks=True,
            disable_semaphore_checks=True,
        ),
        name="adaln_decode",
    )(A_x, c, w_mod, A_wq, A_k_cache, A_v_cache, A_wo.T, B_w3, B_w4.T)
```

```python
import jax
import jax.numpy as jnp
from jax import lax
from jax.experimental import pallas as pl
from jax.experimental.pallas import tpu as pltpu

D, F = 448, 1792
HQ, HKV, DH = 16, 8, 256
WINDOW = 4096
EPS = 1e-5
ROWS = 8
PIECE = 32
BLOCK = 256
BLOCKS = WINDOW // BLOCK
LAG = 4
HEADS = (1, 4, 7, 3, 2, 0, 5, 6)
M_A, M_KV, M_T = 4, 4, 4
W4_GROUPS = (0, 32, 56)
W4_EARLY = (0, 16, 32)
W4_ORDER = ([(r + s, c) for r in range(6, 16) for c in (0, 7) for s in (0, 16)]
            + [(r + s, c) for r in range(9) for c in (0, 7) for s in (38, 47)])
EARLY_MOD, LATE_MOD = 18 * 128, 3 * 128
GATE_ROWS = 16
GATE_ORDER = [i + 9 * s for i in range(9) for s in range(2)] + list(range(18, 28))
GATE_GROUPS = (0, 16, 24, 28)
WM_RUNS = ((7, 4), (11, 7))
W4_FIRST = [54, 55] + [r + s for r in range(12, 18) for s in (0, 18, 36)]
QO_ORDER = (9, 4, 12, 6, 1, 10, 13, 8, 5, 0, 7, 3, 11, 2)
M_L, M_7 = 4, 3
MIX = 0
M_6 = 6
SPLIT = (12, 32, 56, 84)
SKIP = ()
BF16, F32 = jnp.bfloat16, jnp.float32

RING = LAG + 1
S_XC, S_WM, S_WQ, S_WO, S_W3, S_KV = range(6)
S_GATE = S_KV + RING
S_W4 = S_GATE + 4


def _layernorm(x):
    d = x - jnp.sum(x, axis=-1, keepdims=True) * (1.0 / D)
    return d * lax.rsqrt(jnp.sum(d * d, axis=-1, keepdims=True) * (1.0 / D) + EPS)


def _dot(a, b):
    return lax.dot_general(a, b, (((1,), (0,)), ((), ())), preferred_element_type=F32)


def _dot_t(a, b):
    return lax.dot_general(a, b, (((1,), (1,)), ((), ())), preferred_element_type=F32)


def _ds(start, size, align=None):
    return pl.ds(start if isinstance(start, int) else pl.multiple_of(start, align or size), size)


def _loop(lo, hi, body):
    lax.fori_loop(lo, hi, lambda i, carry: body(i), None)


def _kernel(x_hbm, c_hbm, wm_hbm, wq_hbm, k_hbm, v_hbm, wo_hbm, w3_hbm, w4_hbm, out_hbm,
            x_ref, c_ref, wm_ref, wq_ref, k_ref, v_ref, wo_ref, w3_ref, w4_ref,
            mod_ref, wg_ref, col_ref, q_ref, s_ref, max_ref, sum_ref, ctx_ref, acc_ref, hid_ref, out_ref, sems):
    first_key = k_hbm.shape[2] - WINDOW

    def tiles(hbm, ref, sem, row, col, cols, rows=1):
        at = (_ds(row * 8, rows * 8, 8), _ds(col * 128, cols * 128, 128))
        return pltpu.make_async_copy(hbm.at[at], ref.at[at], sems.at[sem])

    def enqueue(copies, every):
        for i, copy in enumerate(copies):
            copy.start(priority=int(i % every != every - 1))

    def landed(ref, sem):
        pltpu.make_async_copy(ref, ref, sems.at[sem]).wait()

    def wide(hbm, ref, sem, i):
        return [tiles(hbm, ref, sem, row + (i >> 2), (i & 3) * 8, 8) for row in range(0, 56, 8)]

    def w_mod_and_w3(i, rows_m, rows_3):
        for (col, cols), half in zip(WM_RUNS, (0, 7)):
            enqueue([tiles(wm_hbm, wm_ref, S_WM, row + i, col, cols) for row in rows_m]
                    + [tiles(w3_hbm, w3_ref, S_W3, row + i, half, 7) for row in rows_3], M_T if len(rows_m) == 5 else M_7)

    def w3_and_w4(i):
        for j in range(2):
            enqueue([tiles(w3_hbm, w3_ref, S_W3, row + 12 + i, 7 * j, 7) for row in (0, 18, 36)]
                    + [tiles(w4_hbm, w4_ref, S_W4 + sum(row >= g for g in W4_GROUPS[1:]), row + i, 7 * j, 7) for row in W4_EARLY], M_6)

    def gate_weights(i):
        return pltpu.make_async_copy(wm_hbm.at[pl.ds(GATE_ROWS * GATE_ORDER[i], GATE_ROWS), pl.ds(EARLY_MOD, LATE_MOD)],
                                     wg_ref.at[pl.ds(GATE_ROWS * i, GATE_ROWS)],
                                     sems.at[S_GATE + sum(i >= g for g in GATE_GROUPS[1:-1])])

    def cache_block(hbm, ref, b, sem, work=lambda i: None):
        start = first_key + b * (BLOCK // 2)
        apart = 3072 - (b >> 3) * 2048

        def body(i):
            enqueue([pltpu.make_async_copy(hbm.at[0, h, _ds(start + s * apart + i * PIECE, PIECE)],
                                           ref.at[b, h, _ds(s * (BLOCK // 2) + i * PIECE, PIECE)], sems.at[sem])
                     for s in range(2) for h in HEADS], M_KV)
            work(i)
        _loop(0, BLOCK // 2 // PIECE, body)

    even = (lax.broadcasted_iota(jnp.int32, (ROWS, DH), 0) & 1) == 0
    small = [pltpu.make_async_copy(c_hbm, c_ref, sems.at[S_XC]), pltpu.make_async_copy(x_hbm, x_ref, sems.at[S_XC])]

    def silu_c():
        c = jnp.broadcast_to(c_ref[...].astype(F32), (ROWS, D))
        return (c * jax.nn.sigmoid(c)).astype(BF16)

    def condition(t):
        both = _dot(silu_c(), wm_ref[:, t * 2 * D:(t + 1) * 2 * D])
        mod_ref[2 * t] = both[:, :D]
        mod_ref[2 * t + 1] = both[:, D:]

    def condition_attention():
        for copy in small:
            copy.wait()
        landed(wm_ref.at[:, :2 * D], S_WM)
        condition(0)

    def attention_input():
        landed(wq_ref, S_WQ)
        x = jnp.broadcast_to(x_ref[0].astype(F32), (ROWS, D))
        acc_ref[...] = _layernorm(x) * (1.0 + mod_ref[1]) + mod_ref[0]

    def queries(h):
        q = _dot(acc_ref[...].astype(BF16), wq_ref[:, _ds(h * 2 * DH, 2 * DH)]) * DH ** -0.5
        q_ref[h] = jnp.where(even, q[:, :DH], q[:, DH:])
        max_ref[h] = jnp.full((ROWS, 128), -jnp.inf, F32)
        sum_ref[h] = jnp.zeros((ROWS, 128), F32)
        ctx_ref[h] = jnp.zeros((ROWS, DH), F32)

    def prepare(i):
        pl.when(i == 4)(condition_attention)
        pl.when(i == 6)(attention_input)
        pl.when((i >= 8) & (i < 16))(lambda: queries(i - 8))

    def scores(b):
        for h in range(HKV):
            s = _dot_t(q_ref[h].astype(BF16), k_ref[b, h])
            s_ref[b, h] = s
            max_ref[h] = jnp.maximum(max_ref[h], jnp.maximum(s[:, :128], s[:, 128:]))

    def row_maxima():
        for h in range(HKV):
            max_ref[h] = jnp.broadcast_to(jnp.max(max_ref[h], axis=-1, keepdims=True), (ROWS, 128))

    def context(b):
        for h in range(HKV):
            p = jnp.exp(s_ref[b, h] - jnp.concatenate([max_ref[h]] * 2, axis=1))
            sum_ref[h] += p[:, :128] + p[:, 128:]
            ctx_ref[h] += _dot(p.astype(BF16), v_ref[b, h])

    def normalize():
        for h in range(HKV):
            ctx_ref[h] = ctx_ref[h] / jnp.sum(sum_ref[h], axis=-1, keepdims=True)
        acc_ref[...] = jnp.zeros((ROWS, D), F32)

    def project(h):
        o = ctx_ref[h]
        o = jnp.concatenate([jnp.where(even, o, 0.0), jnp.where(even, 0.0, o)], axis=1).astype(BF16)
        return _dot_t(o, wo_ref[:, _ds(h * 2 * DH, 2 * DH)])

    _loop(0, 14, lambda i: enqueue([tiles(wm_hbm, wm_ref, S_WM, row + i, 0, 7) for row in (0, 14, 28, 42)], 4))
    enqueue(small, 2)

    def wq_and_wo(i):
        copies = wide(wq_hbm, wq_ref, S_WQ, i) + wide(wo_hbm, wo_ref, S_WO, i)
        enqueue([copies[s] for s in QO_ORDER], M_A)
    _loop(0, 32, wq_and_wo)

    def step(t, slot):
        done = jnp.where(slot == RING - 1, 0, slot + 1)
        pl.when(t < BLOCKS)(lambda: cache_block(k_hbm, k_ref, t, S_KV + slot, lambda i: prepare(4 * t + i)))
        pl.when((t >= BLOCKS) & (t < 2 * BLOCKS))(lambda: cache_block(v_hbm, v_ref, t - BLOCKS, S_KV + slot))
        pl.when(t >= 2 * BLOCKS)(lambda: _loop((t - 2 * BLOCKS) * 2, (t - 2 * BLOCKS + 1) * 2,
                                               lambda i: w_mod_and_w3(i, (0, 12, 24, 36, 48), (0, 18, 36))))

        @pl.when((t >= LAG) & (t < BLOCKS + LAG))
        def _():
            landed(k_ref.at[t - LAG], S_KV + done)
            if 'scores' not in SKIP: scores(t - LAG)

        pl.when(t == BLOCKS + LAG)(row_maxima)

        @pl.when(t >= BLOCKS + LAG)
        def _():
            landed(v_ref.at[t - BLOCKS - LAG], S_KV + done)
            if 'context' not in SKIP: context(t - BLOCKS - LAG)
        return done

    lax.fori_loop(0, 2 * BLOCKS + LAG, step, 0)
    landed(wo_ref, S_WO)
    normalize()

    def output(h):
        pl.when(h < 2)(lambda: enqueue([tiles(w3_hbm, w3_ref, S_W3, 54 + h, 0, 14)], 2))
        pl.when(h < 4)(lambda: w_mod_and_w3(8 + h, (0, 12, 24, 36), (0, 18, 36)))
        pl.when(h >= 4)(lambda: _loop(((h - 4) * 3) >> 1, ((h - 3) * 3) >> 1, w3_and_w4))
        if 'project' not in SKIP: acc_ref[...] += project(h)
    _loop(0, HKV, output)
    last = [tiles(w4_hbm, w4_ref, S_W4 + sum(row >= g for g in W4_GROUPS[1:]), row, col, 7) for row, col in W4_ORDER]
    gates = [gate_weights(i) for i in range(len(GATE_ORDER))]
    last = last[:len(last) - MIX] + [copy for pair in zip(last[len(last) - MIX:], gates) for copy in pair] + gates[MIX:]
    enqueue(last[:20], M_L)
    last = last[20:]
    landed(wm_ref.at[:, 2 * D:], S_WM)
    condition(1)
    c = silu_c()
    rest = _dot(c, wm_ref[:, 4 * D:])
    c = jnp.concatenate([c.astype(F32), jnp.zeros((ROWS, 512 - D), F32)], axis=1)
    for j in range(4):
        col_ref[pl.ds(j * 128, 128)] = jnp.broadcast_to(c[:1, j * 128:(j + 1) * 128], (128, 128)).T
    enqueue(last[:SPLIT[0]], M_L)
    attn = acc_ref[...]
    x = jnp.broadcast_to(x_ref[0].astype(F32), (ROWS, D))
    x = x + mod_ref[2] * (attn + pltpu.roll(attn, 1, 0))
    h_mlp = _layernorm(x) * (1.0 + rest[:, :D]) + mod_ref[3]
    acc_ref[...] = _layernorm(h_mlp)
    enqueue(last[SPLIT[0]:SPLIT[1]], M_L)
    landed(w3_ref, S_W3)
    hid_ref[...] = jax.nn.gelu(_dot(acc_ref[...].astype(BF16), w3_ref[...]), approximate=True)
    enqueue(last[SPLIT[1]:SPLIT[2]], M_L)
    enqueue(last[SPLIT[2]:SPLIT[3]], 99)
    acc_ref[...] = h_mlp
    enqueue(last[SPLIT[3]:], 99)
    for g, (lo, hi) in enumerate(zip(W4_GROUPS, W4_GROUPS[1:])):
        at = pl.ds(lo * 8, (hi - lo) * 8)
        landed(w4_ref.at[at], S_W4 + g)
        if 'w4' not in SKIP: acc_ref[:, at] += _dot_t(hid_ref[...].astype(BF16), w4_ref[at])
    gate = [jnp.zeros((ROWS, 128), F32)] * 3
    for g, (lo, hi) in enumerate(zip(GATE_GROUPS[:-1], GATE_GROUPS[1:])):
        landed(wg_ref.at[pl.ds(lo * GATE_ROWS, (hi - lo) * GATE_ROWS)], S_GATE + g)
        rows = [GATE_ROWS * GATE_ORDER[i] + r for i in range(lo, hi) for r in range(0, GATE_ROWS, 8)]
        for i in range(0, len(rows), 2):
            for j in range(3):
                w = wg_ref[pl.ds(lo * GATE_ROWS + 8 * i, 16), pl.ds(j * 128, 128)].astype(F32)
                gate[j] = gate[j] + (w[:8] * col_ref[pl.ds(rows[i], 8)] + w[8:] * col_ref[pl.ds(rows[i + 1], 8)])
    gate = jnp.concatenate([rest[:1, D:]] + [jnp.sum(part, axis=0, keepdims=True) for part in gate], axis=1)
    if 'gate' in SKIP: gate = 1.0
    out_ref[0] = (x[:1] + gate * acc_ref[:1]).astype(BF16)
    store = pltpu.make_async_copy(out_ref, out_hbm, sems.at[S_XC])
    store.start()
    store.wait()


@jax.jit
def pallas_adaLN_cond__sliding_block_cached__mixer_s_mlp__decode_kernel(
    A_x: jax.Array,
    A_k_cache: jax.Array,
    A_v_cache: jax.Array,
    A_wq: jax.Array,
    A_wo: jax.Array,
    B_x: jax.Array,
    B_w1: jax.Array,
    B_w2: jax.Array,
    B_w3: jax.Array,
    B_w4: jax.Array,
    c: jax.Array,
    w_mod: jax.Array,
):
    keys = A_k_cache.shape[2]
    assert A_x.shape == (1, 1, D) and A_k_cache.shape == (1, HKV, keys, DH)
    assert min(4096, max(256, keys // 4)) == WINDOW and keys % PIECE == 0
    hbm = pl.BlockSpec(memory_space=pltpu.HBM)
    return pl.pallas_call(
        _kernel,
        out_shape=jax.ShapeDtypeStruct(A_x.shape, A_x.dtype),
        in_specs=[hbm] * 9,
        out_specs=hbm,
        scratch_shapes=[
            pltpu.VMEM((1, 1, D), BF16),
            pltpu.VMEM((1, D), BF16),
            pltpu.VMEM((D, EARLY_MOD), BF16),
            pltpu.VMEM((D, HQ * DH), BF16),
            pltpu.VMEM((BLOCKS, HKV, BLOCK, DH), BF16),
            pltpu.VMEM((BLOCKS, HKV, BLOCK, DH), BF16),
            pltpu.VMEM((D, HQ * DH), BF16),
            pltpu.VMEM((D, F), BF16),
            pltpu.VMEM((D, F), BF16),
            pltpu.VMEM((6, ROWS, D), F32),
            pltpu.VMEM((D, LATE_MOD), BF16),
            pltpu.VMEM((512, 128), F32),
            pltpu.VMEM((HKV, ROWS, DH), F32),
            pltpu.VMEM((BLOCKS, HKV, ROWS, BLOCK), F32),
            pltpu.VMEM((HKV, ROWS, 128), F32),
            pltpu.VMEM((HKV, ROWS, 128), F32),
            pltpu.VMEM((HKV, ROWS, DH), F32),
            pltpu.VMEM((ROWS, D), F32),
            pltpu.VMEM((ROWS, F), F32),
            pltpu.VMEM((1, 1, D), BF16),
            pltpu.SemaphoreType.DMA((S_W4 + len(W4_GROUPS) - 1,)),
        ],
        compiler_params=pltpu.CompilerParams(
            vmem_limit_bytes=100 * 2**20,
            disable_bounds_checks=True,
            disable_semaphore_checks=True,
        ),
        name="adaln_decode",
    )(A_x, c, w_mod, A_wq, A_k_cache, A_v_cache, A_wo.T, B_w3, B_w4.T)
```

```python
import jax
import jax.numpy as jnp
from jax import lax
from jax.experimental import pallas as pl
from jax.experimental.pallas import tpu as pltpu

D, F = 448, 1792
HQ, HKV, DH = 16, 8, 256
WINDOW = 4096
EPS = 1e-5
BF16, F32 = jnp.bfloat16, jnp.float32

ROWS = 8
PIECE = 32
BLOCK = 256
BLOCKS = WINDOW // BLOCK
LAG = 4
GATE_COL = 18

K_ROUND = ((2, 8, 14, 6, 4, 0, 10, 12, 3, 9, 15, 7, 5, 1, 11, 13), (3, 7, 11, 15))
V_ROUND = ((2, 8, 14, 6, 4, 0, 10, 12, 3, 9, 15, 7, 5, 1, 11, 13), (3, 7, 11, 15))
WM_ROUND = ((0, 1, 2, 3), (3,))
WQ_WO_ROUND = ((9, 4, 12, 6, 1, 10, 13, 8, 5, 0, 7, 3, 11, 2), (3, 7, 11))
WM5_W3_ROUND = ((0, 1, 2, 3, 4, 5, 6, 7), (3, 7))
WM4_W3_ROUND = ((0, 1, 2, 3, 4, 5, 6), (2, 5))
W3_W4_ROUND = ((0, 1, 2, 3, 4, 5), (5,))
WM_RUNS = ((7, 4), (11, 7))
W4_LATE = ([(r + s, c) for r in range(6, 16) for c in (0, 7) for s in (0, 16)]
           + [(r + s, c) for r in range(9) for c in (0, 7) for s in (38, 47)])
W4_GROUPS = (0, 32, 56)
GATE_ORDER = [i + s for i in range(9) for s in (0, 9)] + list(range(18, 28))
GATE_GROUPS = (0, 18, 25, 28)
LATE_FAST = (4, 76)
LATE_SPLIT = (20, 32, 52)

S_SMALL, S_WM, S_WQ, S_WO, S_W3, S_CACHE = range(6)
S_W4 = S_CACHE + LAG + 1
S_GATE = S_W4 + 3


def _layernorm(x):
    d = x - jnp.sum(x, axis=-1, keepdims=True) * (1.0 / D)
    return d * lax.rsqrt(jnp.sum(d * d, axis=-1, keepdims=True) * (1.0 / D) + EPS)


def _dot(a, b):
    return lax.dot_general(a, b, (((1,), (0,)), ((), ())), preferred_element_type=F32)


def _dot_t(a, b):
    return lax.dot_general(a, b, (((1,), (1,)), ((), ())), preferred_element_type=F32)


def _ds(start, size, align=None):
    return pl.ds(start if isinstance(start, int) else pl.multiple_of(start, align or size), size)


def _loop(lo, hi, body):
    lax.fori_loop(lo, hi, lambda i, carry: body(i), None)


def _kernel(x_hbm, c_hbm, wm_hbm, wq_hbm, k_hbm, v_hbm, wo_hbm, w3_hbm, w4_hbm, out_hbm,
            x_ref, c_ref, wm_ref, wg_ref, wq_ref, k_ref, v_ref, wo_ref, w3_ref, w4_ref,
            mod_ref, col_ref, q_ref, s_ref, max_ref, sum_ref, ctx_ref, acc_ref, hid_ref, out_ref, sems):
    def tiles(hbm, ref, sem, row, col, cols):
        at = (_ds(row * 8, 8), _ds(col * 128, cols * 128, 128))
        return pltpu.make_async_copy(hbm.at[at], ref.at[at], sems.at[sem])

    def enqueue(copies, order, fast):
        for i, j in enumerate(order):
            copies[j].start(priority=int(i not in fast))

    def landed(ref, sem):
        pltpu.make_async_copy(ref, ref, sems.at[sem]).wait()

    def w4_piece(row, i, col):
        return tiles(w4_hbm, w4_ref, S_W4 + sum(row >= g for g in W4_GROUPS[1:]), row + i, col, 7)

    def gate_piece(i):
        return pltpu.make_async_copy(wm_hbm.at[pl.ds(16 * GATE_ORDER[i], 16), GATE_COL * 128:],
                                     wg_ref.at[pl.ds(16 * i, 16)],
                                     sems.at[S_GATE + sum(i >= g for g in GATE_GROUPS[1:])])

    def wq_and_wo(i):
        enqueue([tiles(hbm, ref, sem, row + (i >> 2), (i & 3) * 8, 8)
                 for hbm, ref, sem in ((wq_hbm, wq_ref, S_WQ), (wo_hbm, wo_ref, S_WO))
                 for row in range(0, 56, 8)], *WQ_WO_ROUND)

    def wm_and_w3(i, wm_rows, round_):
        for (col, cols), half in zip(WM_RUNS, (0, 7)):
            enqueue([tiles(wm_hbm, wm_ref, S_WM, row + i, col, cols) for row in wm_rows]
                    + [tiles(w3_hbm, w3_ref, S_W3, row + i, half, 7) for row in (0, 18, 36)], *round_)

    def w3_and_w4(i):
        for half in (0, 7):
            enqueue([tiles(w3_hbm, w3_ref, S_W3, row + i, half, 7) for row in (12, 30, 48)]
                    + [w4_piece(row, i, half) for row in (0, 16, 32)], *W3_W4_ROUND)

    def cache_block(hbm, ref, b, sem, round_, work=lambda i: None):
        start = hbm.shape[2] - WINDOW + b * (BLOCK // 2)
        apart = 3072 - (b >> 3) * 2048

        def body(i):
            enqueue([pltpu.make_async_copy(hbm.at[0, h, _ds(start + s * apart + i * PIECE, PIECE)],
                                           ref.at[b, h, _ds(s * (BLOCK // 2) + i * PIECE, PIECE)], sems.at[sem])
                     for h in range(HKV) for s in range(2)], *round_)
            work(i)
        _loop(0, BLOCK // 2 // PIECE, body)

    small = [pltpu.make_async_copy(c_hbm, c_ref, sems.at[S_SMALL]),
             pltpu.make_async_copy(x_hbm, x_ref, sems.at[S_SMALL])]

    def even_rows():
        return (lax.broadcasted_iota(jnp.int32, (ROWS, DH), 0) & 1) == 0

    def silu_c():
        c = jnp.broadcast_to(c_ref[...].astype(F32), (ROWS, D))
        return (c * jax.nn.sigmoid(c)).astype(BF16)

    def modulation(t):
        both = _dot(silu_c(), wm_ref[:, t * 2 * D:(t + 1) * 2 * D])
        mod_ref[2 * t] = both[:, :D]
        mod_ref[2 * t + 1] = both[:, D:]

    def attention_modulation():
        for copy in small:
            copy.wait()
        landed(wm_ref.at[:, :2 * D], S_WM)
        modulation(0)

    def attention_input():
        landed(wq_ref, S_WQ)
        x = jnp.broadcast_to(x_ref[0].astype(F32), (ROWS, D))
        acc_ref[...] = _layernorm(x) * (1.0 + mod_ref[1]) + mod_ref[0]

    def queries(h):
        q = _dot(acc_ref[...].astype(BF16), wq_ref[:, _ds(h * 2 * DH, 2 * DH)]) * DH ** -0.5
        q_ref[h] = jnp.where(even_rows(), q[:, :DH], q[:, DH:])
        max_ref[h] = jnp.full((ROWS, 128), -jnp.inf, F32)
        sum_ref[h] = jnp.zeros((ROWS, 128), F32)
        ctx_ref[h] = jnp.zeros((ROWS, DH), F32)

    def prepare(i):
        pl.when(i == 4)(attention_modulation)
        pl.when(i == 6)(attention_input)
        pl.when((i >= 8) & (i < 8 + HKV))(lambda: queries(i - 8))

    def scores(b):
        for h in range(HKV):
            s = _dot_t(q_ref[h].astype(BF16), k_ref[b, h])
            s_ref[b, h] = s
            max_ref[h] = jnp.maximum(max_ref[h], jnp.maximum(s[:, :128], s[:, 128:]))

    def row_maxima():
        for h in range(HKV):
            max_ref[h] = jnp.broadcast_to(jnp.max(max_ref[h], axis=-1, keepdims=True), (ROWS, 128))

    def context(b):
        for h in range(HKV):
            p = jnp.exp(s_ref[b, h] - jnp.concatenate([max_ref[h]] * 2, axis=1))
            sum_ref[h] += p[:, :128] + p[:, 128:]
            ctx_ref[h] += _dot(p.astype(BF16), v_ref[b, h])

    def normalize():
        for h in range(HKV):
            ctx_ref[h] = ctx_ref[h] / jnp.sum(sum_ref[h], axis=-1, keepdims=True)
        acc_ref[...] = jnp.zeros((ROWS, D), F32)

    def project(h):
        o, even = ctx_ref[h], even_rows()
        o = jnp.concatenate([jnp.where(even, o, 0.0), jnp.where(even, 0.0, o)], axis=1).astype(BF16)
        return _dot_t(o, wo_ref[:, _ds(h * 2 * DH, 2 * DH)])

    _loop(0, 14, lambda i: enqueue([tiles(wm_hbm, wm_ref, S_WM, row + i, 0, 7) for row in range(0, 56, 14)],
                                   *WM_ROUND))
    enqueue(small, (0, 1), (1,))
    _loop(0, 32, wq_and_wo)

    def step(t, slot):
        done = jnp.where(slot == LAG, 0, slot + 1)

        @pl.when(t < BLOCKS)
        def _():
            cache_block(k_hbm, k_ref, t, S_CACHE + slot, K_ROUND, lambda i: prepare(4 * t + i))

        @pl.when((t >= BLOCKS) & (t < 2 * BLOCKS))
        def _():
            cache_block(v_hbm, v_ref, t - BLOCKS, S_CACHE + slot, V_ROUND)

        @pl.when(t >= 2 * BLOCKS)
        def _():
            first = 2 * (t - 2 * BLOCKS)
            _loop(first, first + 2, lambda i: wm_and_w3(i, (0, 12, 24, 36, 48), WM5_W3_ROUND))

        @pl.when((t >= LAG) & (t < BLOCKS + LAG))
        def _():
            landed(k_ref.at[t - LAG], S_CACHE + done)
            scores(t - LAG)

        pl.when(t == BLOCKS + LAG)(row_maxima)

        @pl.when(t >= BLOCKS + LAG)
        def _():
            landed(v_ref.at[t - BLOCKS - LAG], S_CACHE + done)
            context(t - BLOCKS - LAG)
        return done

    lax.fori_loop(0, 2 * BLOCKS + LAG, step, 0)
    landed(wo_ref, S_WO)
    normalize()

    def output(h):
        pl.when(h < 2)(lambda: tiles(w3_hbm, w3_ref, S_W3, 54 + h, 0, 14).start(priority=1))
        pl.when(h < 4)(lambda: wm_and_w3(8 + h, (0, 12, 24, 36), WM4_W3_ROUND))
        pl.when(h >= 4)(lambda: _loop((3 * h - 12) >> 1, (3 * h - 9) >> 1, w3_and_w4))
        acc_ref[...] += project(h)
    _loop(0, HKV, output)

    late = [w4_piece(row, 0, col) for row, col in W4_LATE] + [gate_piece(i) for i in range(len(GATE_ORDER))]
    every, until = LATE_FAST

    def enqueue_late(lo, hi):
        enqueue(late, range(lo, hi), [i - lo for i in range(every - 1, until, every)])

    enqueue_late(0, LATE_SPLIT[0])
    landed(wm_ref.at[:, 2 * D:], S_WM)
    modulation(1)
    c = silu_c()
    rest = _dot(c, wm_ref[:, 4 * D:])
    c = jnp.concatenate([c.astype(F32), jnp.zeros((ROWS, 512 - D), F32)], axis=1)
    for j in range(4):
        col_ref[pl.ds(j * 128, 128)] = jnp.broadcast_to(c[:1, j * 128:(j + 1) * 128], (128, 128)).T
    enqueue_late(LATE_SPLIT[0], LATE_SPLIT[1])
    attn = acc_ref[...]
    x = jnp.broadcast_to(x_ref[0].astype(F32), (ROWS, D))
    x = x + mod_ref[2] * (attn + pltpu.roll(attn, 1, 0))
    h_mlp = _layernorm(x) * (1.0 + rest[:, :D]) + mod_ref[3]
    acc_ref[...] = _layernorm(h_mlp)
    enqueue_late(LATE_SPLIT[1], LATE_SPLIT[2])
    landed(w3_ref, S_W3)
    hid_ref[...] = jax.nn.gelu(_dot(acc_ref[...].astype(BF16), w3_ref[...]), approximate=True)
    acc_ref[...] = h_mlp
    enqueue_late(LATE_SPLIT[2], len(late))
    for g, (lo, hi) in enumerate(zip(W4_GROUPS, W4_GROUPS[1:])):
        at = pl.ds(lo * 8, (hi - lo) * 8)
        landed(w4_ref.at[at], S_W4 + g)
        acc_ref[:, at] += _dot_t(hid_ref[...].astype(BF16), w4_ref[at])

    gate = [jnp.zeros((ROWS, 128), F32)] * 3
    for g, (lo, hi) in enumerate(zip(GATE_GROUPS, GATE_GROUPS[1:])):
        landed(wg_ref.at[pl.ds(lo * 16, (hi - lo) * 16)], S_GATE + g)
        for i in range(lo, hi):
            col = col_ref[pl.ds(16 * GATE_ORDER[i], 16)]
            for j in range(3):
                prod = wg_ref[pl.ds(16 * i, 16), pl.ds(128 * j, 128)].astype(F32) * col
                gate[j] = gate[j] + (prod[:8] + prod[8:])
    gate = jnp.concatenate([rest[:1, D:]] + [jnp.sum(part, axis=0, keepdims=True) for part in gate], axis=1)
    out_ref[0] = (x[:1] + gate * acc_ref[:1]).astype(BF16)
    store = pltpu.make_async_copy(out_ref, out_hbm, sems.at[S_SMALL])
    store.start()
    store.wait()


@jax.jit
def pallas_adaLN_cond__sliding_block_cached__mixer_s_mlp__decode_kernel(
    A_x: jax.Array,
    A_k_cache: jax.Array,
    A_v_cache: jax.Array,
    A_wq: jax.Array,
    A_wo: jax.Array,
    B_x: jax.Array,
    B_w1: jax.Array,
    B_w2: jax.Array,
    B_w3: jax.Array,
    B_w4: jax.Array,
    c: jax.Array,
    w_mod: jax.Array,
):
    keys = A_k_cache.shape[2]
    assert A_x.shape == (1, 1, D) and A_k_cache.shape == (1, HKV, keys, DH)
    assert min(4096, max(256, keys // 4)) == WINDOW and keys % PIECE == 0
    hbm = pl.BlockSpec(memory_space=pltpu.HBM)
    return pl.pallas_call(
        _kernel,
        out_shape=jax.ShapeDtypeStruct(A_x.shape, A_x.dtype),
        in_specs=[hbm] * 9,
        out_specs=hbm,
        scratch_shapes=[
            pltpu.VMEM((1, 1, D), BF16),
            pltpu.VMEM((1, D), BF16),
            pltpu.VMEM((D, GATE_COL * 128), BF16),
            pltpu.VMEM((D, 6 * D - GATE_COL * 128), BF16),
            pltpu.VMEM((D, HQ * DH), BF16),
            pltpu.VMEM((BLOCKS, HKV, BLOCK, DH), BF16),
            pltpu.VMEM((BLOCKS, HKV, BLOCK, DH), BF16),
            pltpu.VMEM((D, HQ * DH), BF16),
            pltpu.VMEM((D, F), BF16),
            pltpu.VMEM((D, F), BF16),
            pltpu.VMEM((4, ROWS, D), F32),
            pltpu.VMEM((512, 128), F32),
            pltpu.VMEM((HKV, ROWS, DH), F32),
            pltpu.VMEM((BLOCKS, HKV, ROWS, BLOCK), F32),
            pltpu.VMEM((HKV, ROWS, 128), F32),
            pltpu.VMEM((HKV, ROWS, 128), F32),
            pltpu.VMEM((HKV, ROWS, DH), F32),
            pltpu.VMEM((ROWS, D), F32),
            pltpu.VMEM((ROWS, F), F32),
            pltpu.VMEM((1, 1, D), BF16),
            pltpu.SemaphoreType.DMA((S_GATE + len(GATE_GROUPS) - 1,)),
        ],
        compiler_params=pltpu.CompilerParams(
            vmem_limit_bytes=100 * 2**20,
            disable_bounds_checks=True,
            disable_semaphore_checks=True,
        ),
        name="adaln_decode",
    )(A_x, c, w_mod, A_wq, A_k_cache, A_v_cache, A_wo.T, B_w3, B_w4.T)
```

```python
import jax
import jax.numpy as jnp
from jax import lax
from jax.experimental import pallas as pl
from jax.experimental.pallas import tpu as pltpu

D, F = 448, 1792
HQ, HKV, DH = 16, 8, 256
WINDOW = 4096
EPS = 1e-5
BF16, F32 = jnp.bfloat16, jnp.float32

ROWS = 8
PIECE = 32
BLOCK = 256
BLOCKS = WINDOW // BLOCK
LAG = 4
GATE_COL = 18

K_ROUND = ((0, 10, 7, 5, 13, 2, 8, 15, 3, 9, 4, 6, 14, 1, 11, 12), (3, 7, 11, 15))
V_ROUND = ((0, 10, 1, 4, 11, 6, 12, 14, 7, 13, 2, 5, 8, 3, 9, 15), (3, 7, 11, 15))
WM_ROUND = ((3, 1, 2, 0), (3,))
WQ_WO_ROUND = ((7, 13, 4, 11, 2, 3, 6, 10, 12, 1, 8, 9, 0, 5), (2, 6, 9, 13))
WM5_W3_ROUND = ((0, 1, 2, 3, 4, 5, 6, 7), (3, 7))
WM4_W3_ROUND = ((0, 1, 2, 3, 4, 5, 6), (3,))
W3_W4_ROUND = ((0, 1, 2, 3, 4, 5), (5,))
WM_RUNS = ((7, 6), (13, 5))
W4_LATE = ([(r + s, c) for r in range(5) for c in (0, 7) for s in (6, 22, 11, 27)]
           + [(r + s, c) for r in range(9) for c in (0, 7) for s in (38, 47)])
W4_GROUPS = (0, 32, 56)
GATE_GROUPS = (0, 16, 24, 28)
LATE_FAST = range(3, 52, 4)
LATE_SPLIT = (16, 36, 60)

S_SMALL, S_WM, S_WQ, S_WO, S_W3, S_CACHE = range(6)
S_W4 = S_CACHE + LAG + 1
S_GATE = S_W4 + 3


def _layernorm(x):
    d = x - jnp.sum(x, axis=-1, keepdims=True) * (1.0 / D)
    return d * lax.rsqrt(jnp.sum(d * d, axis=-1, keepdims=True) * (1.0 / D) + EPS)


def _dot(a, b):
    return lax.dot_general(a, b, (((1,), (0,)), ((), ())), preferred_element_type=F32)


def _dot_t(a, b):
    return lax.dot_general(a, b, (((1,), (1,)), ((), ())), preferred_element_type=F32)


def _ds(start, size, align=None):
    return pl.ds(start if isinstance(start, int) else pl.multiple_of(start, align or size), size)


def _loop(lo, hi, body):
    lax.fori_loop(lo, hi, lambda i, carry: body(i), None)


def _kernel(x_hbm, c_hbm, wm_hbm, wq_hbm, k_hbm, v_hbm, wo_hbm, w3_hbm, w4_hbm, out_hbm,
            x_ref, c_ref, wm_ref, wg_ref, wq_ref, k_ref, v_ref, wo_ref, w3_ref, w4_ref,
            mod_ref, col_ref, q_ref, s_ref, max_ref, sum_ref, ctx_ref, acc_ref, hid_ref, out_ref, sems):
    def tiles(hbm, ref, sem, row, col, cols):
        at = (_ds(row * 8, 8), _ds(col * 128, cols * 128, 128))
        return pltpu.make_async_copy(hbm.at[at], ref.at[at], sems.at[sem])

    def enqueue(copies, order, fast):
        for i, j in enumerate(order):
            copies[j].start(priority=int(i not in fast))

    def landed(ref, sem):
        pltpu.make_async_copy(ref, ref, sems.at[sem]).wait()

    def w4_piece(row, i, col):
        return tiles(w4_hbm, w4_ref, S_W4 + sum(row >= g for g in W4_GROUPS[1:]), row + i, col, 7)

    def gate_piece(i):
        return pltpu.make_async_copy(wm_hbm.at[pl.ds(16 * i, 16), GATE_COL * 128:], wg_ref.at[pl.ds(16 * i, 16)],
                                     sems.at[S_GATE + sum(i >= g for g in GATE_GROUPS[1:])])

    def wq_and_wo(i):
        enqueue([tiles(hbm, ref, sem, row + (i >> 2), (i & 3) * 8, 8)
                 for hbm, ref, sem in ((wq_hbm, wq_ref, S_WQ), (wo_hbm, wo_ref, S_WO))
                 for row in range(0, 56, 8)], *WQ_WO_ROUND)

    def wm_and_w3(i, wm_rows, round_):
        for (col, cols), half in zip(WM_RUNS, (0, 7)):
            enqueue([tiles(wm_hbm, wm_ref, S_WM, row + i, col, cols) for row in wm_rows]
                    + [tiles(w3_hbm, w3_ref, S_W3, row + i, half, 7) for row in (0, 18, 36)], *round_)

    def w3_and_w4(i):
        for half in (0, 7):
            enqueue([tiles(w3_hbm, w3_ref, S_W3, row + i, half, 7) for row in (12, 30, 48)]
                    + [w4_piece(row, i, half) for row in (0, 16, 32)], *W3_W4_ROUND)

    def cache_block(hbm, ref, b, sem, round_, work=lambda i: None):
        start = hbm.shape[2] - WINDOW + b * (BLOCK // 2)
        apart = 3072 - (b >> 3) * 2048

        def body(i):
            enqueue([pltpu.make_async_copy(hbm.at[0, h, _ds(start + s * apart + i * PIECE, PIECE)],
                                           ref.at[b, h, _ds(s * (BLOCK // 2) + i * PIECE, PIECE)], sems.at[sem])
                     for h in range(HKV) for s in range(2)], *round_)
            work(i)
        _loop(0, BLOCK // 2 // PIECE, body)

    small = [pltpu.make_async_copy(c_hbm, c_ref, sems.at[S_SMALL]),
             pltpu.make_async_copy(x_hbm, x_ref, sems.at[S_SMALL])]

    def even_rows():
        return (lax.broadcasted_iota(jnp.int32, (ROWS, DH), 0) & 1) == 0

    def silu_c():
        c = jnp.broadcast_to(c_ref[...].astype(F32), (ROWS, D))
        return (c * jax.nn.sigmoid(c)).astype(BF16)

    def modulation(t):
        both = _dot(silu_c(), wm_ref[:, t * 2 * D:(t + 1) * 2 * D])
        mod_ref[2 * t] = both[:, :D]
        mod_ref[2 * t + 1] = both[:, D:]

    def attention_modulation():
        for copy in small:
            copy.wait()
        landed(wm_ref.at[:, :2 * D], S_WM)
        modulation(0)

    def attention_input():
        landed(wq_ref, S_WQ)
        x = jnp.broadcast_to(x_ref[0].astype(F32), (ROWS, D))
        acc_ref[...] = _layernorm(x) * (1.0 + mod_ref[1]) + mod_ref[0]

    def queries(h):
        q = _dot(acc_ref[...].astype(BF16), wq_ref[:, _ds(h * 2 * DH, 2 * DH)]) * DH ** -0.5
        q_ref[h] = jnp.where(even_rows(), q[:, :DH], q[:, DH:])
        max_ref[h] = jnp.full((ROWS, 128), -jnp.inf, F32)
        sum_ref[h] = jnp.zeros((ROWS, 128), F32)
        ctx_ref[h] = jnp.zeros((ROWS, DH), F32)

    def prepare(i):
        pl.when(i == 4)(attention_modulation)
        pl.when(i == 6)(attention_input)
        pl.when((i >= 8) & (i < 8 + HKV))(lambda: queries(i - 8))

    def scores(b):
        for h in range(HKV):
            s = _dot_t(q_ref[h].astype(BF16), k_ref[b, h])
            s_ref[b, h] = s
            max_ref[h] = jnp.maximum(max_ref[h], jnp.maximum(s[:, :128], s[:, 128:]))

    def row_maxima():
        for h in range(HKV):
            max_ref[h] = jnp.broadcast_to(jnp.max(max_ref[h], axis=-1, keepdims=True), (ROWS, 128))

    def context(b):
        for h in range(HKV):
            p = jnp.exp(s_ref[b, h] - jnp.concatenate([max_ref[h]] * 2, axis=1))
            sum_ref[h] += p[:, :128] + p[:, 128:]
            ctx_ref[h] += _dot(p.astype(BF16), v_ref[b, h])

    def normalize():
        for h in range(HKV):
            ctx_ref[h] = ctx_ref[h] / jnp.sum(sum_ref[h], axis=-1, keepdims=True)
        acc_ref[...] = jnp.zeros((ROWS, D), F32)

    def project(h):
        o, even = ctx_ref[h], even_rows()
        o = jnp.concatenate([jnp.where(even, o, 0.0), jnp.where(even, 0.0, o)], axis=1).astype(BF16)
        return _dot_t(o, wo_ref[:, _ds(h * 2 * DH, 2 * DH)])

    _loop(0, 14, lambda i: enqueue([tiles(wm_hbm, wm_ref, S_WM, row + i, 0, 7) for row in range(0, 56, 14)],
                                   *WM_ROUND))
    enqueue(small, (0, 1), (1,))
    _loop(0, 32, wq_and_wo)

    def step(t, slot):
        done = jnp.where(slot == LAG, 0, slot + 1)

        @pl.when(t < BLOCKS)
        def _():
            cache_block(k_hbm, k_ref, t, S_CACHE + slot, K_ROUND, lambda i: prepare(4 * t + i))

        @pl.when((t >= BLOCKS) & (t < 2 * BLOCKS))
        def _():
            cache_block(v_hbm, v_ref, t - BLOCKS, S_CACHE + slot, V_ROUND)

        @pl.when(t >= 2 * BLOCKS)
        def _():
            first = 2 * (t - 2 * BLOCKS)
            _loop(first, first + 2, lambda i: wm_and_w3(i, (0, 12, 24, 36, 48), WM5_W3_ROUND))

        @pl.when((t >= LAG) & (t < BLOCKS + LAG))
        def _():
            landed(k_ref.at[t - LAG], S_CACHE + done)
            scores(t - LAG)

        pl.when(t == BLOCKS + LAG)(row_maxima)

        @pl.when(t >= BLOCKS + LAG)
        def _():
            landed(v_ref.at[t - BLOCKS - LAG], S_CACHE + done)
            context(t - BLOCKS - LAG)
        return done

    lax.fori_loop(0, 2 * BLOCKS + LAG, step, 0)
    landed(wo_ref, S_WO)
    normalize()

    def output(h):
        pl.when(h < 2)(lambda: tiles(w3_hbm, w3_ref, S_W3, 54 + h, 0, 14).start(priority=1))
        pl.when(h < 4)(lambda: wm_and_w3(8 + h, (0, 12, 24, 36), WM4_W3_ROUND))
        pl.when(h >= 4)(lambda: _loop((3 * h - 12) >> 1, (3 * h - 9) >> 1, w3_and_w4))
        acc_ref[...] += project(h)
    _loop(0, HKV, output)

    late = [w4_piece(row, 0, col) for row, col in W4_LATE] + [gate_piece(i) for i in range(D // 16)]

    def enqueue_late(lo, hi):
        enqueue(late, range(lo, hi), [i - lo for i in LATE_FAST])

    enqueue_late(0, LATE_SPLIT[0])
    landed(wm_ref.at[:, 2 * D:], S_WM)
    modulation(1)
    c = silu_c()
    rest = _dot(c, wm_ref[:, 4 * D:])
    c = jnp.concatenate([c.astype(F32), jnp.zeros((ROWS, 512 - D), F32)], axis=1)
    for j in range(4):
        col_ref[pl.ds(j * 128, 128)] = jnp.broadcast_to(c[:1, j * 128:(j + 1) * 128], (128, 128)).T
    enqueue_late(LATE_SPLIT[0], LATE_SPLIT[1])
    attn = acc_ref[...]
    x = jnp.broadcast_to(x_ref[0].astype(F32), (ROWS, D))
    x = x + mod_ref[2] * (attn + pltpu.roll(attn, 1, 0))
    h_mlp = _layernorm(x) * (1.0 + rest[:, :D]) + mod_ref[3]
    acc_ref[...] = _layernorm(h_mlp)
    enqueue_late(LATE_SPLIT[1], LATE_SPLIT[2])
    landed(w3_ref, S_W3)
    hid_ref[...] = jax.nn.gelu(_dot(acc_ref[...].astype(BF16), w3_ref[...]), approximate=True)
    acc_ref[...] = h_mlp
    enqueue_late(LATE_SPLIT[2], len(late))
    for g, (lo, hi) in enumerate(zip(W4_GROUPS, W4_GROUPS[1:])):
        at = pl.ds(lo * 8, (hi - lo) * 8)
        landed(w4_ref.at[at], S_W4 + g)
        acc_ref[:, at] += _dot_t(hid_ref[...].astype(BF16), w4_ref[at])

    gate = [jnp.zeros((ROWS, 128), F32)] * 3
    for g, (lo, hi) in enumerate(zip(GATE_GROUPS, GATE_GROUPS[1:])):
        landed(wg_ref.at[pl.ds(lo * 16, (hi - lo) * 16)], S_GATE + g)
        for i in range(lo, hi):
            col = col_ref[pl.ds(16 * i, 16)]
            for j in range(3):
                prod = wg_ref[pl.ds(16 * i, 16), pl.ds(128 * j, 128)].astype(F32) * col
                gate[j] = gate[j] + (prod[:8] + prod[8:])
    gate = jnp.concatenate([rest[:1, D:]] + [jnp.sum(part, axis=0, keepdims=True) for part in gate], axis=1)
    out_ref[0] = (x[:1] + gate * acc_ref[:1]).astype(BF16)
    store = pltpu.make_async_copy(out_ref, out_hbm, sems.at[S_SMALL])
    store.start()
    store.wait()


@jax.jit
def pallas_adaLN_cond__sliding_block_cached__mixer_s_mlp__decode_kernel(
    A_x: jax.Array,
    A_k_cache: jax.Array,
    A_v_cache: jax.Array,
    A_wq: jax.Array,
    A_wo: jax.Array,
    B_x: jax.Array,
    B_w1: jax.Array,
    B_w2: jax.Array,
    B_w3: jax.Array,
    B_w4: jax.Array,
    c: jax.Array,
    w_mod: jax.Array,
):
    keys = A_k_cache.shape[2]
    assert A_x.shape == (1, 1, D) and A_k_cache.shape == (1, HKV, keys, DH)
    assert min(4096, max(256, keys // 4)) == WINDOW and keys % PIECE == 0
    hbm = pl.BlockSpec(memory_space=pltpu.HBM)
    return pl.pallas_call(
        _kernel,
        out_shape=jax.ShapeDtypeStruct(A_x.shape, A_x.dtype),
        in_specs=[hbm] * 9,
        out_specs=hbm,
        scratch_shapes=[
            pltpu.VMEM((1, 1, D), BF16),
            pltpu.VMEM((1, D), BF16),
            pltpu.VMEM((D, GATE_COL * 128), BF16),
            pltpu.VMEM((D, 6 * D - GATE_COL * 128), BF16),
            pltpu.VMEM((D, HQ * DH), BF16),
            pltpu.VMEM((BLOCKS, HKV, BLOCK, DH), BF16),
            pltpu.VMEM((BLOCKS, HKV, BLOCK, DH), BF16),
            pltpu.VMEM((D, HQ * DH), BF16),
            pltpu.VMEM((D, F), BF16),
            pltpu.VMEM((D, F), BF16),
            pltpu.VMEM((4, ROWS, D), F32),
            pltpu.VMEM((512, 128), F32),
            pltpu.VMEM((HKV, ROWS, DH), F32),
            pltpu.VMEM((BLOCKS, HKV, ROWS, BLOCK), F32),
            pltpu.VMEM((HKV, ROWS, 128), F32),
            pltpu.VMEM((HKV, ROWS, 128), F32),
            pltpu.VMEM((HKV, ROWS, DH), F32),
            pltpu.VMEM((ROWS, D), F32),
            pltpu.VMEM((ROWS, F), F32),
            pltpu.VMEM((1, 1, D), BF16),
            pltpu.SemaphoreType.DMA((S_GATE + len(GATE_GROUPS) - 1,)),
        ],
        compiler_params=pltpu.CompilerParams(
            vmem_limit_bytes=100 * 2**20,
            disable_bounds_checks=True,
            disable_semaphore_checks=True,
        ),
        name="adaln_decode",
    )(A_x, c, w_mod, A_wq, A_k_cache, A_v_cache, A_wo.T, B_w3, B_w4.T)
```

```python
import jax
import jax.numpy as jnp
from jax import lax
from jax.experimental import pallas as pl
from jax.experimental.pallas import tpu as pltpu

D, F = 448, 1792
HQ, HKV, DH = 16, 8, 256
WINDOW = 4096
EPS = 1e-5
BF16, F32 = jnp.bfloat16, jnp.float32

ROWS = 8
PIECE = 32
BLOCK = 256
BLOCKS = WINDOW // BLOCK
LAG = 4
GATE_COL = 18

CACHE_ROUND = ((4, 14, 2, 5, 15, 0, 10, 8, 1, 11, 3, 6, 12, 7, 13, 9), (2, 7, 10, 15))
WQ_WO_ROUND = ((3, 10, 4, 13, 8, 12, 6, 0, 2, 1, 11, 7, 9, 5), (2, 6, 9, 13))
WM5_W3_ROUND = ((0, 1, 2, 3, 4, 5, 6, 7), (3, 7))
WM4_W3_ROUND = ((0, 1, 2, 3, 4, 5, 6), (3,))
W3_W4_ROUND = ((0, 1, 2, 3, 4, 5), (5,))
WM_RUNS = ((7, 6), (13, 5))
W4_LATE = ([(r + s, c) for r in range(5) for c in (0, 7) for s in (6, 22, 11, 27)]
           + [(r + s, c) for r in range(9) for c in (0, 7) for s in (38, 47)])
W4_GROUPS = (0, 32, 56)
GATE_GROUPS = (0, 16, 24, 28)
LATE_FAST = range(3, 52, 4)
LATE_SPLIT = (16, 36, 60)

S_SMALL, S_WM, S_WQ, S_WO, S_W3, S_CACHE = range(6)
S_W4 = S_CACHE + LAG + 1
S_GATE = S_W4 + len(W4_GROUPS) - 1


def _layernorm(x):
    d = x - jnp.sum(x, axis=-1, keepdims=True) * (1.0 / D)
    return d * lax.rsqrt(jnp.sum(d * d, axis=-1, keepdims=True) * (1.0 / D) + EPS)


def _dot(a, b):
    return lax.dot_general(a, b, (((1,), (0,)), ((), ())), preferred_element_type=F32)


def _dot_t(a, b):
    return lax.dot_general(a, b, (((1,), (1,)), ((), ())), preferred_element_type=F32)


def _ds(start, size, align=None):
    return pl.ds(start if isinstance(start, int) else pl.multiple_of(start, align or size), size)


def _loop(lo, hi, body):
    lax.fori_loop(lo, hi, lambda i, carry: body(i), None)


def _kernel(x_hbm, c_hbm, wm_hbm, wq_hbm, k_hbm, v_hbm, wo_hbm, w3_hbm, w4_hbm, out_hbm,
            x_ref, c_ref, wm_ref, wg_ref, wq_ref, k_ref, v_ref, wo_ref, w3_ref, w4_ref,
            mod_ref, col_ref, q_ref, s_ref, max_ref, sum_ref, ctx_ref, acc_ref, hid_ref, out_ref, sems):
    def tiles(hbm, ref, sem, row, col, cols):
        at = (_ds(row * 8, 8), _ds(col * 128, cols * 128, 128))
        return pltpu.make_async_copy(hbm.at[at], ref.at[at], sems.at[sem])

    def enqueue(copies, order, fast):
        for i, j in enumerate(order):
            copies[j].start(priority=int(i not in fast))

    def landed(ref, sem):
        pltpu.make_async_copy(ref, ref, sems.at[sem]).wait()

    def w4_piece(row, i, col):
        return tiles(w4_hbm, w4_ref, S_W4 + sum(row >= g for g in W4_GROUPS[1:]), row + i, col, 7)

    def gate_piece(i):
        return pltpu.make_async_copy(wm_hbm.at[pl.ds(16 * i, 16), GATE_COL * 128:], wg_ref.at[pl.ds(16 * i, 16)],
                                     sems.at[S_GATE + sum(i >= g for g in GATE_GROUPS[1:])])

    def wm_alone(i, rows):
        enqueue([tiles(wm_hbm, wm_ref, S_WM, row + i, 0, 7) for row in rows], range(len(rows)), (len(rows) - 1,))

    def wq_and_wo(i):
        enqueue([tiles(hbm, ref, sem, row + (i >> 2), (i & 3) * 8, 8)
                 for hbm, ref, sem in ((wq_hbm, wq_ref, S_WQ), (wo_hbm, wo_ref, S_WO))
                 for row in range(0, 56, 8)], *WQ_WO_ROUND)

    def wm_and_w3(i, wm_rows, round_):
        for (col, cols), half in zip(WM_RUNS, (0, 7)):
            enqueue([tiles(wm_hbm, wm_ref, S_WM, row + i, col, cols) for row in wm_rows]
                    + [tiles(w3_hbm, w3_ref, S_W3, row + i, half, 7) for row in (0, 18, 36)], *round_)

    def w3_and_w4(i):
        for half in (0, 7):
            enqueue([tiles(w3_hbm, w3_ref, S_W3, row + i, half, 7) for row in (12, 30, 48)]
                    + [w4_piece(row, i, half) for row in (0, 16, 32)], *W3_W4_ROUND)

    def cache_block(hbm, ref, b, sem, work=lambda i: None):
        start = hbm.shape[2] - WINDOW + b * (BLOCK // 2) + (b >> 3) * (WINDOW // 4)

        def body(i):
            enqueue([pltpu.make_async_copy(hbm.at[0, h, _ds(start + s * (WINDOW // 4) + i * PIECE, PIECE)],
                                           ref.at[b, h, _ds(s * (BLOCK // 2) + i * PIECE, PIECE)], sems.at[sem])
                     for h in range(HKV) for s in range(2)], *CACHE_ROUND)
            work(i)
        _loop(0, BLOCK // 2 // PIECE, body)

    small = [pltpu.make_async_copy(c_hbm, c_ref, sems.at[S_SMALL]),
             pltpu.make_async_copy(x_hbm, x_ref, sems.at[S_SMALL])]

    def even_rows():
        return (lax.broadcasted_iota(jnp.int32, (ROWS, DH), 0) & 1) == 0

    def silu_c():
        c = jnp.broadcast_to(c_ref[...].astype(F32), (ROWS, D))
        return (c * jax.nn.sigmoid(c)).astype(BF16)

    def modulation(t):
        both = _dot(silu_c(), wm_ref[:, t * 2 * D:(t + 1) * 2 * D])
        mod_ref[2 * t] = both[:, :D]
        mod_ref[2 * t + 1] = both[:, D:]

    def attention_modulation():
        for copy in small:
            copy.wait()
        landed(wm_ref.at[:, :2 * D], S_WM)
        modulation(0)

    def attention_input():
        landed(wq_ref, S_WQ)
        x = jnp.broadcast_to(x_ref[0].astype(F32), (ROWS, D))
        acc_ref[...] = _layernorm(x) * (1.0 + mod_ref[1]) + mod_ref[0]

    def queries(h):
        q = _dot(acc_ref[...].astype(BF16), wq_ref[:, _ds(h * 2 * DH, 2 * DH)]) * DH ** -0.5
        q_ref[h] = jnp.where(even_rows(), q[:, :DH], q[:, DH:])
        max_ref[h] = jnp.full((ROWS, 128), -jnp.inf, F32)
        sum_ref[h] = jnp.zeros((ROWS, 128), F32)
        ctx_ref[h] = jnp.zeros((ROWS, DH), F32)

    def prepare(i):
        pl.when(i == 4)(attention_modulation)
        pl.when(i == 6)(attention_input)
        pl.when((i >= 8) & (i < 8 + HKV))(lambda: queries(i - 8))

    def scores(b):
        for h in range(HKV):
            s = _dot_t(q_ref[h].astype(BF16), k_ref[b, h])
            s_ref[b, h] = s
            max_ref[h] = jnp.maximum(max_ref[h], jnp.maximum(s[:, :128], s[:, 128:]))

    def row_maxima():
        for h in range(HKV):
            max_ref[h] = jnp.broadcast_to(jnp.max(max_ref[h], axis=-1, keepdims=True), (ROWS, 128))

    def context(b):
        for h in range(HKV):
            p = jnp.exp(s_ref[b, h] - jnp.concatenate([max_ref[h]] * 2, axis=1))
            sum_ref[h] += p[:, :128] + p[:, 128:]
            ctx_ref[h] += _dot(p.astype(BF16), v_ref[b, h])

    def normalize():
        for h in range(HKV):
            ctx_ref[h] = ctx_ref[h] / jnp.sum(sum_ref[h], axis=-1, keepdims=True)
        acc_ref[...] = jnp.zeros((ROWS, D), F32)

    def project(h):
        o, even = ctx_ref[h], even_rows()
        o = jnp.concatenate([jnp.where(even, o, 0.0), jnp.where(even, 0.0, o)], axis=1).astype(BF16)
        return _dot_t(o, wo_ref[:, _ds(h * 2 * DH, 2 * DH)])

    wm_alone(0, (0, 12, 24, 36, 48))
    _loop(1, 8, lambda i: wm_alone(i, (0, 12, 24, 36, 48)))
    _loop(8, 12, lambda i: wm_alone(i, (0, 12, 24, 36)))
    enqueue(small, (0, 1), (1,))
    _loop(0, 32, wq_and_wo)

    def step(t, slot):
        done = jnp.where(slot == LAG, 0, slot + 1)

        @pl.when(t < BLOCKS)
        def _():
            cache_block(k_hbm, k_ref, t, S_CACHE + slot, lambda i: prepare(4 * t + i))

        @pl.when((t >= BLOCKS) & (t < 2 * BLOCKS))
        def _():
            cache_block(v_hbm, v_ref, t - BLOCKS, S_CACHE + slot)

        @pl.when(t >= 2 * BLOCKS)
        def _():
            first = 2 * (t - 2 * BLOCKS)
            _loop(first, first + 2, lambda i: wm_and_w3(i, (0, 12, 24, 36, 48), WM5_W3_ROUND))

        @pl.when((t >= LAG) & (t < BLOCKS + LAG))
        def _():
            landed(k_ref.at[t - LAG], S_CACHE + done)
            scores(t - LAG)

        pl.when(t == BLOCKS + LAG)(row_maxima)

        @pl.when(t >= BLOCKS + LAG)
        def _():
            landed(v_ref.at[t - BLOCKS - LAG], S_CACHE + done)
            context(t - BLOCKS - LAG)
        return done

    lax.fori_loop(0, 2 * BLOCKS + LAG, step, 0)
    landed(wo_ref, S_WO)
    normalize()

    def output(h):
        pl.when(h < 2)(lambda: tiles(w3_hbm, w3_ref, S_W3, 54 + h, 0, 14).start(priority=1))
        pl.when(h < 4)(lambda: wm_and_w3(8 + h, (0, 12, 24, 36), WM4_W3_ROUND))
        pl.when(h >= 4)(lambda: _loop((3 * h - 12) >> 1, (3 * h - 9) >> 1, w3_and_w4))
        acc_ref[...] += project(h)
    _loop(0, HKV, output)

    late = [w4_piece(row, 0, col) for row, col in W4_LATE] + [gate_piece(i) for i in range(D // 16)]

    def enqueue_late(lo, hi):
        enqueue(late, range(lo, hi), [i - lo for i in LATE_FAST])

    enqueue_late(0, LATE_SPLIT[0])
    landed(wm_ref.at[:, 2 * D:], S_WM)
    modulation(1)
    c = silu_c()
    rest = _dot(c, wm_ref[:, 4 * D:])
    c = jnp.concatenate([c.astype(F32), jnp.zeros((ROWS, 512 - D), F32)], axis=1)
    for j in range(4):
        col_ref[pl.ds(j * 128, 128)] = jnp.broadcast_to(c[:1, j * 128:(j + 1) * 128], (128, 128)).T
    enqueue_late(LATE_SPLIT[0], LATE_SPLIT[1])
    attn = acc_ref[...]
    x = jnp.broadcast_to(x_ref[0].astype(F32), (ROWS, D))
    x = x + mod_ref[2] * (attn + pltpu.roll(attn, 1, 0))
    h_mlp = _layernorm(x) * (1.0 + rest[:, :D]) + mod_ref[3]
    acc_ref[...] = _layernorm(h_mlp)
    enqueue_late(LATE_SPLIT[1], LATE_SPLIT[2])
    landed(w3_ref, S_W3)
    hid_ref[...] = jax.nn.gelu(_dot(acc_ref[...].astype(BF16), w3_ref[...]), approximate=True)
    acc_ref[...] = h_mlp
    enqueue_late(LATE_SPLIT[2], len(late))
    for g, (lo, hi) in enumerate(zip(W4_GROUPS, W4_GROUPS[1:])):
        at = pl.ds(lo * 8, (hi - lo) * 8)
        landed(w4_ref.at[at], S_W4 + g)
        acc_ref[:, at] += _dot_t(hid_ref[...].astype(BF16), w4_ref[at])

    gate = [jnp.zeros((ROWS, 128), F32)] * 3
    for g, (lo, hi) in enumerate(zip(GATE_GROUPS, GATE_GROUPS[1:])):
        landed(wg_ref.at[pl.ds(lo * 16, (hi - lo) * 16)], S_GATE + g)
        for i in range(lo, hi):
            col = col_ref[pl.ds(16 * i, 16)]
            for j in range(3):
                prod = wg_ref[pl.ds(16 * i, 16), pl.ds(128 * j, 128)].astype(F32) * col
                gate[j] = gate[j] + (prod[:8] + prod[8:])
    gate = jnp.concatenate([rest[:1, D:]] + [jnp.sum(part, axis=0, keepdims=True) for part in gate], axis=1)
    out_ref[0] = (x[:1] + gate * acc_ref[:1]).astype(BF16)
    store = pltpu.make_async_copy(out_ref, out_hbm, sems.at[S_SMALL])
    store.start()
    store.wait()


@jax.jit
def pallas_adaLN_cond__sliding_block_cached__mixer_s_mlp__decode_kernel(
    A_x: jax.Array,
    A_k_cache: jax.Array,
    A_v_cache: jax.Array,
    A_wq: jax.Array,
    A_wo: jax.Array,
    B_x: jax.Array,
    B_w1: jax.Array,
    B_w2: jax.Array,
    B_w3: jax.Array,
    B_w4: jax.Array,
    c: jax.Array,
    w_mod: jax.Array,
):
    keys = A_k_cache.shape[2]
    assert A_x.shape == (1, 1, D) and A_k_cache.shape == (1, HKV, keys, DH)
    assert min(4096, max(256, keys // 4)) == WINDOW and keys % PIECE == 0
    hbm = pl.BlockSpec(memory_space=pltpu.HBM)
    return pl.pallas_call(
        _kernel,
        out_shape=jax.ShapeDtypeStruct(A_x.shape, A_x.dtype),
        in_specs=[hbm] * 9,
        out_specs=hbm,
        scratch_shapes=[
            pltpu.VMEM((1, 1, D), BF16),
            pltpu.VMEM((1, D), BF16),
            pltpu.VMEM((D, GATE_COL * 128), BF16),
            pltpu.VMEM((D, 6 * D - GATE_COL * 128), BF16),
            pltpu.VMEM((D, HQ * DH), BF16),
            pltpu.VMEM((BLOCKS, HKV, BLOCK, DH), BF16),
            pltpu.VMEM((BLOCKS, HKV, BLOCK, DH), BF16),
            pltpu.VMEM((D, HQ * DH), BF16),
            pltpu.VMEM((D, F), BF16),
            pltpu.VMEM((D, F), BF16),
            pltpu.VMEM((4, ROWS, D), F32),
            pltpu.VMEM((512, 128), F32),
            pltpu.VMEM((HKV, ROWS, DH), F32),
            pltpu.VMEM((BLOCKS, HKV, ROWS, BLOCK), F32),
            pltpu.VMEM((HKV, ROWS, 128), F32),
            pltpu.VMEM((HKV, ROWS, 128), F32),
            pltpu.VMEM((HKV, ROWS, DH), F32),
            pltpu.VMEM((ROWS, D), F32),
            pltpu.VMEM((ROWS, F), F32),
            pltpu.VMEM((1, 1, D), BF16),
            pltpu.SemaphoreType.DMA((S_GATE + len(GATE_GROUPS) - 1,)),
        ],
        compiler_params=pltpu.CompilerParams(
            vmem_limit_bytes=100 * 2**20,
            disable_bounds_checks=True,
            disable_semaphore_checks=True,
        ),
        name="adaln_decode",
    )(A_x, c, w_mod, A_wq, A_k_cache, A_v_cache, A_wo.T, B_w3, B_w4.T)
```
